```python
import jax
import jax.numpy as jnp

def _softmax(x, axis=-1):
    return jax.nn.softmax(x, axis=axis)
def _gelu(x):
    return jax.nn.gelu(x, approximate=True)
def _silu(x):
    return jax.nn.silu(x)
def _sigmoid(x):
    return jax.nn.sigmoid(x)
def _layernorm(x, axis=-1, eps=1e-5):
    m = jnp.mean(x, axis=axis, keepdims=True)
    v = jnp.var(x, axis=axis, keepdims=True)
    return (x - m) / jnp.sqrt(v + eps)
def _scatter_add(tgt, idx, src, axis=0):
    return tgt.at[idx].add(src)
def _segment_sum(src, seg, n):
    return jax.ops.segment_sum(src, seg, n)
class _Rng:
    def __init__(self, key):
        self._k = key
    def _next(self):
        self._k, sub = jax.random.split(self._k)
        return sub
    def normal(self, shape):
        return jax.random.normal(self._next(), shape, dtype=jnp.bfloat16)
    def randint(self, lo, hi, shape):
        return jax.random.randint(self._next(), shape, lo, hi, dtype=jnp.int32)
    def uniform(self, shape, lo=0.0, hi=1.0):
        return jax.random.uniform(self._next(), shape, jnp.bfloat16, lo, hi)
    def permutation(self, n):
        return jax.random.permutation(self._next(), n)


kernel_name = 'interleave_layers__sliding_block_cached__dense_activation_gelu__decode'

def setup_inputs():
    _rng = _Rng(jax.random.key(int.from_bytes(__import__("os").urandom(4), "little")))
    _w = (lambda a: (lambda t: t.astype(jnp.bfloat16) if jnp.issubdtype(t.dtype, jnp.floating) else t)(jnp.asarray(a)))
    def _A_setup():
        B, Sq, D = 1, 1, 640
        Hq, Hkv, Sk, Dh = 32, 32, 32768, 192
        assert Hq % Hkv == 0, (Hq, Hkv)
        return {
            "x": _w((lambda *s: _rng.normal(s) * 0.05)(B, Sq, D)),
            "k_cache": _w((lambda *s: _rng.normal(s) * 0.05)(B, Hkv, Sk, Dh)),
            "v_cache": _w((lambda *s: _rng.normal(s) * 0.05)(B, Hkv, Sk, Dh)),
            "wq": _w((lambda *s: _rng.normal(s) * 0.05)(D, Hq * Dh) * (D ** -0.5)),
            "wo": _w((lambda *s: _rng.normal(s) * 0.05)(Hq * Dh, D) * ((Hq * Dh) ** -0.5)),
        }
    _A_in = _A_setup()

    def _B_setup():
        B, S, D, F = 1, 1, 640, 1536
        return {
            "x": _w((lambda *s: _rng.normal(s) * 0.05)(B, S, D)),
            "w1": _w((lambda *s: _rng.normal(s) * 0.05)(D, F) * (D ** -0.5)),
            "b1": _w((lambda *s: _rng.normal(s) * 0.05)(F) * 0.01),
            "w2": _w((lambda *s: _rng.normal(s) * 0.05)(F, D) * (F ** -0.5)),
            "b2": _w((lambda *s: _rng.normal(s) * 0.05)(D) * 0.01),
        }
    _B_in = _B_setup()

    return {
        "A_x": _A_in["x"],
        "A_k_cache": _A_in["k_cache"],
        "A_v_cache": _A_in["v_cache"],
        "A_wq": _A_in["wq"],
        "A_wo": _A_in["wo"],
        "B_x": _B_in["x"],
        "B_w1": _B_in["w1"],
        "B_b1": _B_in["b1"],
        "B_w2": _B_in["w2"],
        "B_b2": _B_in["b2"],
    }

def reference(A_x, A_k_cache, A_v_cache, A_wq, A_wo, B_x, B_w1, B_b1, B_w2, B_b2):
    def _A_ref(x, k_cache, v_cache, wq, wo):
        B, Sq, D = x.shape
        Hq, Dh = 32, 192
        Hkv, Sk = k_cache.shape[1], k_cache.shape[2]
        W = min(4096, max(256, Sk // 4))
        rep = Hq // Hkv
        q = (lambda x, *d: x.transpose(*d))((x @ wq).reshape(B, Sq, Hq, Dh), 0, 2, 1, 3)
        k = jnp.repeat(k_cache[:, :, Sk - W:, :], rep, axis=1)
        v = jnp.repeat(v_cache[:, :, Sk - W:, :], rep, axis=1)
        scores = jnp.einsum("bhqd,bhkd->bhqk", q, k) * (Dh ** -0.5)
        p = _softmax(scores, axis=-1)
        o = jnp.einsum("bhqk,bhkd->bhqd", p, v)
        return (lambda x, *d: x.transpose(*d))(o, 0, 2, 1, 3).reshape(B, Sq, Hq * Dh) @ wo

    def _B_ref(x, w1, b1, w2, b2):
        h = jnp.einsum("bsd,df->bsf", x, w1) + b1
        h = _gelu(h)
        return jnp.einsum("bsf,fd->bsd", h, w2) + b2

    x = A_x
    x = x + _A_ref(_layernorm(x, axis=-1), A_k_cache, A_v_cache, A_wq, A_wo)
    x = x + _B_ref(_layernorm(x, axis=-1), B_w1, B_b1, B_w2, B_b2)
    x = x + _A_ref(_layernorm(x, axis=-1), A_k_cache, A_v_cache, A_wq, A_wo)
    x = x + _B_ref(_layernorm(x, axis=-1), B_w1, B_b1, B_w2, B_b2)
    return x
```

```python
import numpy as np
import jax
import jax.numpy as jnp
from jax import lax
import jax.experimental.pallas as pl
import jax.experimental.pallas.tpu as pltpu

F32 = jnp.float32
BF16 = jnp.bfloat16
U32 = jnp.uint32

D = 640
H = 32
DH = 192
FF = 1536
NP = H // 2
PW = 2 * DH
G = PW // 16
UNROLL = 2
CHUNKS = (8, 4, 2, 2)
W2_CHUNKS = 2
LAG = 2


def _bf(w):
    return pltpu.bitcast(w, BF16)


def _layernorm(x):
    m = jnp.mean(x, axis=-1, keepdims=True)
    c = x - m
    v = jnp.mean(c * c, axis=-1, keepdims=True)
    return c / jnp.sqrt(v + 1e-5)


def _make_kernel(sk, win):
    nt = win // 128
    starts = [int(s) for s in np.cumsum((0,) + CHUNKS[:-1])]
    nch = len(CHUNKS)
    f2 = FF // W2_CHUNKS

    def kernel(x_hbm, k_hbm, v_hbm, wq_hbm, wo_hbm, w1_hbm, b1_hbm, w2_hbm, b2_hbm,
               o_ref,
               kbuf, vbuf, wqb, wob, w1b, w2b, xb, b1b, b2b,
               qb, sb, pb, ab, zb, sems):
        sem_idx = [0]

        def copy(src, dst):
            c = pltpu.make_async_copy(src, dst, sems.at[sem_idx[0]])
            sem_idx[0] += 1
            return c

        def halves(src, dst, g0, ng, cols):
            s = src.bitcast(U32)
            return [copy(s.at[pl.ds(g0, ng), hf, :, cols],
                         dst.at[pl.ds(g0, ng), pl.ds(4 * hf, 4), :]) for hf in range(2)]

        window = pl.ds(sk - win, win)
        c_wq = halves(wq_hbm, wqb, 0, D // 16, pl.ds(0, H * DH))
        c_small = [copy(x_hbm, xb), copy(b1_hbm, b1b), copy(b2_hbm, b2b)]
        c_k, c_vo = [], []
        for s0, n in zip(starts, CHUNKS):
            c_k.append(halves(k_hbm, kbuf, s0 * G, n * G, window))
            c_vo.append(halves(v_hbm, vbuf, s0 * G, n * G, window)
                        + halves(wo_hbm, wob, s0 * G, n * G, pl.ds(0, D)))
        c_w1 = copy(w1_hbm, w1b)
        c_w2 = [copy(w2_hbm.at[pl.ds(i * f2, f2)], w2b.at[pl.ds(i * f2, f2)])
                for i in range(W2_CHUNKS)]

        for c in c_wq + c_small:
            c.start()
        for ck, cv in zip(c_k, c_vo):
            for c in ck + cv:
                c.start()
        c_w1.start()
        for c in c_w2:
            c.start()

        def wait(cs):
            for c in cs:
                c.wait()

        zb[...] = jnp.zeros(zb.shape, F32)
        ab[...] = jnp.zeros(ab.shape, F32)

        scale = np.float32(DH ** -0.5)
        row = lax.broadcasted_iota(jnp.int32, (8, PW), 0)
        lane = lax.broadcasted_iota(jnp.int32, (8, PW), 1)
        bd = ((row == 0) & (lane < DH)) | ((row == 1) & (lane >= DH))

        def q_proj(xn, j, slot):
            cols = pl.ds(pl.multiple_of(j * PW, 128), PW)
            w = _bf(wqb[:, :, cols].reshape(D // 2, PW))
            q = jnp.dot(xn, w, preferred_element_type=F32)
            qb[slot] = jnp.where(bd, q, 0.0)
            return q[:, :128]

        def qk_tile(q, j, t, slot):
            kk = _bf(kbuf[pl.ds(j * G, G), :, t * 128:(t + 1) * 128].reshape(PW // 2, 128))
            s = jnp.dot(q, kk, preferred_element_type=F32)
            sb[slot, :, t * 128:(t + 1) * 128] = s
            return s

        def out_proj(y, l, j, slot, valid=None):
            cols = []
            for c in range(PW // 128):
                a = ab[slot, c * 128:(c + 1) * 128, :].T
                a = jnp.sum(a.reshape(16, 8, 128), axis=0)
                cols.append(jnp.broadcast_to(jnp.sum(a, axis=0, keepdims=True), (8, 128)))
            o = jnp.concatenate(cols, axis=1) / l
            m = bd if valid is None else bd & valid
            o = jnp.where(m, o, 0.0).astype(BF16)
            w = _bf(wob[pl.ds(j * G, G)].reshape(PW // 2, D))
            return y + jnp.dot(o, w, preferred_element_type=F32)

        def step(xn, i, slot, m, l_prev, y, flag, first):
            q = qb[1 - slot].astype(BF16)
            jn = jnp.minimum(i + 1, NP - 1)
            lacc = [None]

            def exp_tile(t):
                p = jnp.exp((sb[slot, :, t * 128:(t + 1) * 128] - m) * scale)
                pb[:, t * 128:(t + 1) * 128] = p
                lacc[0] = p if lacc[0] is None else lacc[0] + p

            exp_tile(0)
            exp_tile(1)
            ss = []
            mx = None
            accs = [None] * 24
            extra = {}
            for t in range(nt):
                s = qk_tile(q, jn, t, 1 - slot)
                mx = s if mx is None else jnp.maximum(mx, s)
                ss.append(s)
                if t == nt // 3:
                    valid = (i > 0) if first else None
                    y = out_proj(y, l_prev, jnp.maximum(i - 1, 0), 1 - slot, valid)
                    extra[t + 6] = y[:, :128]
                if t == 2 * nt // 3:
                    extra[t + 6] = q_proj(xn, jnp.minimum(i + 2, NP - 1), slot)
                for u in range(2):
                    h, tt = divmod(2 * t + u, nt)
                    if h == 0 and tt + 2 < nt:
                        exp_tile(tt + 2)
                    p = jnp.broadcast_to(pb[pl.ds(h, 1), tt * 128:(tt + 1) * 128], (8, 128))
                    if u == 0 and t >= LAG:
                        p = jnp.where(flag, ss[t - LAG], p)
                    if u == 1 and t in extra:
                        p = jnp.where(flag, extra[t], p)
                    for g in range(G // 2):
                        f = _bf(vbuf[i * G + h * (G // 2) + g, :, tt * 128:(tt + 1) * 128]).astype(F32)
                        a, b = f[:8] * p, f[8:] * p
                        accs[2 * g] = a if tt == 0 else accs[2 * g] + a
                        accs[2 * g + 1] = b if tt == 0 else accs[2 * g + 1] + b
                    if tt == nt - 1:
                        ab[slot, h * DH:(h + 1) * DH, :] = jnp.concatenate(accs, axis=0)
            m_next = jnp.max(mx, axis=-1, keepdims=True)
            l = jnp.sum(lacc[0], axis=-1, keepdims=True)
            return m_next, l, y

        def layer(li, x):
            first_layer = li == 0
            xn = _layernorm(x).astype(BF16)
            q_proj(xn, 0, 0)
            q_proj(xn, 1, 1)

            @pl.when(first_layer)
            def _():
                wait(c_k[0] + c_vo[0])

            q0 = qb[0].astype(BF16)
            mx = None
            for t in range(nt):
                s = qk_tile(q0, 0, t, 0)
                mx = s if mx is None else jnp.maximum(mx, s)
            m0 = jnp.max(mx, axis=-1, keepdims=True)

            def body(it, carry):
                m, l, y = carry
                i0 = it * UNROLL

                @pl.when(first_layer)
                def _():
                    for c in range(1, nch):
                        @pl.when(i0 + UNROLL == starts[c])
                        def _():
                            wait(c_k[c])

                        @pl.when(i0 == starts[c])
                        def _():
                            wait(c_vo[c])

                flag = zb[...] > 0.0
                for u in range(UNROLL):
                    m, l, y = step(xn, i0 + u, u % 2, m, l, y, flag, u == 0)
                return m, l, y

            _, l, y = lax.fori_loop(
                0, NP // UNROLL, body,
                (m0, jnp.ones((8, 1), F32), jnp.zeros((8, D), F32)))
            y = out_proj(y, l, NP - 1, (NP - 1) % 2)
            x = x + jnp.sum(y, axis=0, keepdims=True)

            xn2 = _layernorm(x).astype(BF16)

            @pl.when(first_layer)
            def _():
                c_w1.wait()

            hid = jnp.dot(xn2, w1b[...], preferred_element_type=F32)
            hid = hid + b1b[...].astype(F32).reshape(1, FF)
            hid = jax.nn.gelu(hid, approximate=True).astype(BF16)
            x = x + b2b[...].astype(F32).reshape(1, D)
            for c in range(W2_CHUNKS):
                @pl.when(first_layer)
                def _():
                    c_w2[c].wait()

                x = x + jnp.dot(hid[:, c * f2:(c + 1) * f2], w2b[c * f2:(c + 1) * f2, :],
                                preferred_element_type=F32)
            return x

        wait(c_small + c_wq)
        x0 = jnp.broadcast_to(xb[...].astype(F32), (8, D))
        xf = lax.fori_loop(0, 2, layer, x0)
        o_ref[...] = xf[0:1].astype(o_ref.dtype)

    n_sems = 2 + 3 + 6 * nch + 1 + W2_CHUNKS
    return kernel, n_sems


@jax.jit
def pallas_interleave_layers__sliding_block_cached__dense_activation_gelu__decode_kernel(
    A_x: jax.Array,
    A_k_cache: jax.Array,
    A_v_cache: jax.Array,
    A_wq: jax.Array,
    A_wo: jax.Array,
    B_x: jax.Array,
    B_w1: jax.Array,
    B_b1: jax.Array,
    B_w2: jax.Array,
    B_b2: jax.Array,
):
    del B_x
    sk = A_k_cache.shape[2]
    win = min(4096, max(256, sk // 4))
    rows = H * DH
    kt = jnp.swapaxes(A_k_cache, 2, 3).reshape(rows // 16, 2, 8, sk)
    vt = jnp.swapaxes(A_v_cache, 2, 3).reshape(rows // 16, 2, 8, sk)
    wq = A_wq.reshape(D // 16, 2, 8, rows)
    wo = A_wo.reshape(rows // 16, 2, 8, D)
    kernel, n_sems = _make_kernel(sk, win)
    out = pl.pallas_call(
        kernel,
        out_shape=jax.ShapeDtypeStruct((1, D), A_x.dtype),
        in_specs=[pl.BlockSpec(memory_space=pl.ANY)] * 9,
        out_specs=pl.BlockSpec(memory_space=pltpu.VMEM),
        scratch_shapes=[
            pltpu.VMEM((rows // 16, 8, win), U32),
            pltpu.VMEM((rows // 16, 8, win), U32),
            pltpu.VMEM((D // 16, 8, rows), U32),
            pltpu.VMEM((rows // 16, 8, D), U32),
            pltpu.VMEM((D, FF), BF16),
            pltpu.VMEM((FF, D), BF16),
            pltpu.VMEM((1, D), BF16),
            pltpu.VMEM((FF,), BF16),
            pltpu.VMEM((D,), BF16),
            pltpu.VMEM((2, 8, PW), F32),
            pltpu.VMEM((2, 8, win), F32),
            pltpu.VMEM((8, win), F32),
            pltpu.VMEM((2, PW, 128), F32),
            pltpu.VMEM((8, 128), F32),
            pltpu.SemaphoreType.DMA((n_sems,)),
        ],
        compiler_params=pltpu.CompilerParams(vmem_limit_bytes=126 * 2**20),
        name="attn_ffn_decode",
    )(A_x.reshape(1, D), kt, vt, wq, wo, B_w1, B_b1, B_w2, B_b2)
    return out.reshape(A_x.shape)
```

```python
import numpy as np
import jax
import jax.numpy as jnp
from jax import lax
import jax.experimental.pallas as pl
import jax.experimental.pallas.tpu as pltpu

F32 = jnp.float32
BF16 = jnp.bfloat16
U32 = jnp.uint32

D = 640
H = 32
DH = 192
FF = 1536
NP = H // 2
PW = 2 * DH
G = PW // 16
UNROLL = 2
CHUNKS = (8, 4, 2, 2)
W2_CHUNKS = 2
LAG = 1000
GATE = 4
EXP_AHEAD = 8
PASSES = 12
TAIL = 45
BARRIER = True
LOG2E = np.float32(np.log2(np.e))


def _bf(w):
    return pltpu.bitcast(w, BF16)


def _layernorm(x):
    m = jnp.mean(x, axis=-1, keepdims=True)
    c = x - m
    v = jnp.mean(c * c, axis=-1, keepdims=True)
    return c / jnp.sqrt(v + 1e-5)


def _make_kernel(sk, win):
    nt = win // 128
    starts = [int(s) for s in np.cumsum((0,) + CHUNKS[:-1])]
    nch = len(CHUNKS)
    f2 = FF // W2_CHUNKS

    def kernel(x_hbm, k_hbm, v_hbm, wq_hbm, wo_hbm, w1_hbm, b1_hbm, w2_hbm, b2_hbm,
               o_ref,
               kbuf, vbuf, wqb, wob, w1b, w2b, xb, b1b, b2b,
               q0, q1, s0_, s1_, p0, p1, a0, a1, m0, m1, l0, l1, zb, yb, one, sems):
        qb, sb, pb, ab, mb, lb = (q0, q1), (s0_, s1_), (p0, p1), (a0, a1), (m0, m1), (l0, l1)
        sem_idx = [0]

        def copy(src, dst):
            c = pltpu.make_async_copy(src, dst, sems.at[sem_idx[0]])
            sem_idx[0] += 1
            return c

        def halves(src, dst, g0, ng, cols):
            s = src.bitcast(U32)
            return [copy(s.at[pl.ds(g0, ng), hf, :, cols],
                         dst.at[pl.ds(g0, ng), pl.ds(4 * hf, 4), :]) for hf in range(2)]

        window = pl.ds(sk - win, win)
        c_wq = halves(wq_hbm, wqb, 0, D // 16, pl.ds(0, H * DH))
        c_small = [copy(x_hbm, xb), copy(b1_hbm, b1b), copy(b2_hbm, b2b)]
        c_k, c_vo = [], []
        for s0, n in zip(starts, CHUNKS):
            c_k.append(halves(k_hbm, kbuf, s0 * G, n * G, window))
            c_vo.append(halves(v_hbm, vbuf, s0 * G, n * G, window)
                        + halves(wo_hbm, wob, s0 * G, n * G, pl.ds(0, D)))
        c_w1 = copy(w1_hbm, w1b)
        c_w2 = [copy(w2_hbm.at[pl.ds(i * f2, f2)], w2b.at[pl.ds(i * f2, f2)])
                for i in range(W2_CHUNKS)]

        for c in c_wq + c_small:
            c.start()
        for ck, cv in zip(c_k, c_vo):
            for c in ck + cv:
                c.start()
        c_w1.start()
        for c in c_w2:
            c.start()

        def wait(cs):
            for c in cs:
                c.wait()

        zb[...] = jnp.zeros(zb.shape, F32)
        a1[...] = jnp.zeros(a1.shape, F32)
        l1[...] = jnp.ones(l1.shape, F32)
        for u in range(2 * UNROLL):
            one[u] = 1

        scale = np.float32(DH ** -0.5)
        row = lax.broadcasted_iota(jnp.int32, (8, PW), 0)
        lane = lax.broadcasted_iota(jnp.int32, (8, PW), 1)
        bd = ((row == 0) & (lane < DH)) | ((row == 1) & (lane >= DH))

        def q_proj(xn, j, slot):
            cols = pl.ds(pl.multiple_of(j * PW, 128), PW)
            w = _bf(wqb[:, :, cols].reshape(D // 2, PW))
            q = jnp.dot(xn, w, preferred_element_type=F32)
            qb[slot][...] = jnp.where(bd, q, 0.0)
            return q[:, PW - 128:]

        def qk_tile(q, j, t, slot):
            kk = _bf(kbuf[pl.ds(j * G, G), :, t * 128:(t + 1) * 128].reshape(PW // 2, 128))
            s = jnp.dot(q, kk, preferred_element_type=F32)[:8]
            sb[slot][:, t * 128:(t + 1) * 128] = s
            return s

        def out_proj(y, l, j, slot, valid=None):
            cols = []
            for c in range(PW // 128):
                a = ab[slot][c * 128:(c + 1) * 128, :].T
                a = jnp.sum(a.reshape(16, 8, 128), axis=0)
                cols.append(jnp.broadcast_to(jnp.sum(a, axis=0, keepdims=True), (8, 128)))
            o = jnp.concatenate(cols, axis=1) / jnp.sum(l, axis=-1, keepdims=True)
            m = bd if valid is None else bd & valid
            o = jnp.where(m, o, 0.0).astype(BF16)
            w = _bf(wob[pl.ds(j * G, G)].reshape(PW // 2, D))
            return y + jnp.dot(o, w, preferred_element_type=F32)

        def pair_step(xn, i, slot, first):
            flag = zb[...] > 0.0
            hist = []

            def gated(v, pos):
                if pos <= GATE:
                    return v
                st["n"] += 1
                a = hist[pos - 1 - GATE]
                g = jnp.where(flag, pltpu.bitcast(a[st["n"] % len(a)], v.dtype), v[:8, :128])
                if v.shape[1] > 128:
                    return jnp.concatenate([g, v[:, 128:]], axis=1)
                return jnp.concatenate([g, v[8:]], axis=0)

            def pack(v):
                return pltpu.bitcast(jnp.concatenate([v, v], axis=0).astype(BF16), U32)

            def mm(lhs, w, pos):
                return jnp.dot(_bf(gated(lhs, pos)), _bf(w), preferred_element_type=F32)[:8]

            m = jnp.max(mb[slot][...], axis=-1, keepdims=True)
            st = dict(n=0, l=None, mx=None, cols=[], q=pack(qb[1 - slot][...]))
            jk = jnp.minimum(i + 1, NP - 1)
            jq = jnp.minimum(i + 2, NP - 1)
            jo = jnp.maximum(i - 1, 0)

            def exp_tile(t):
                p = jnp.exp2((sb[slot][:, t * 128:(t + 1) * 128] - m) * (scale * LOG2E))
                pb[slot][:, t * 128:(t + 1) * 128] = p
                st["l"] = p if st["l"] is None else st["l"] + p

            def job_qk(t, pos):
                w = kbuf[pl.ds(jk * G, G), :, t * 128:(t + 1) * 128].reshape(PW // 2, 128)
                sc = mm(st["q"], w, pos)
                sb[1 - slot][:, t * 128:(t + 1) * 128] = sc
                st["mx"] = sc if st["mx"] is None else jnp.maximum(st["mx"], sc)
                return sc

            def job_q(c, pos):
                cols = pl.ds(pl.multiple_of(jq * PW + c * 128, 128), 128)
                q = mm(xn, wqb[:, :, cols].reshape(D // 2, 128), pos)
                qb[slot][:, c * 128:(c + 1) * 128] = jnp.where(bd[:, c * 128:(c + 1) * 128], q, 0.0)
                return q

            def job_t(c, pos):
                a = gated(ab[1 - slot][c * 128:(c + 1) * 128, :], pos).T
                a = jnp.sum(a.reshape(16, 8, 128), axis=0)
                a = jnp.broadcast_to(jnp.sum(a, axis=0, keepdims=True), (8, 128))
                st["cols"].append(a)
                if c == PW // 128 - 1:
                    o = jnp.concatenate(st["cols"], axis=1)
                    o = o / jnp.sum(lb[1 - slot][...], axis=-1, keepdims=True)
                    st["o"] = pack(jnp.where(bd & (i > 0) if first else bd, o, 0.0))
                return a

            def job_o(c, pos):
                w = wob[pl.ds(jo * G, G), :, c * 128:(c + 1) * 128].reshape(PW // 2, 128)
                y = mm(st["o"], w, pos)
                yb[:, c * 128:(c + 1) * 128] += y
                return y

            jobs = ([(job_qk, t, 3) for t in range(nt)]
                    + [(job_o, c, 3) for c in range(D // 128)]
                    + [(job_q, c, 5) for c in range(PW // 128)])
            total = sum(j[2] for j in jobs)
            ns = PASSES * nt
            at, done = {}, 0
            for fn, arg, cost in jobs:
                at.setdefault(done * (ns - TAIL) // total, []).append((fn, arg))
                done += cost
            for c in range(PW // 128):
                at.setdefault((2 + c) * ns // 8, []).append((job_t, c))

            for t in range(EXP_AHEAD):
                exp_tile(t)
            gp = G // PASSES
            deps = {}
            for pos in range(ns):
                ps, tt = divmod(pos, nt)
                for fn, arg in at.get(pos, []):
                    deps[pos + LAG] = fn(arg, pos)
                if ps == 0 and tt + EXP_AHEAD < nt:
                    exp_tile(tt + EXP_AHEAD)
                h = ps * 2 // PASSES
                p = jnp.broadcast_to(pb[slot][pl.ds(h, 1), tt * 128:(tt + 1) * 128], (8, 128))
                if pos in deps:
                    p = jnp.where(flag, deps[pos], p)
                if tt == 0:
                    accs = [None] * (2 * gp)
                for g in range(gp):
                    f = _bf(vbuf[i * G + ps * gp + g, :, tt * 128:(tt + 1) * 128]).astype(F32)
                    a, b = f[:8] * p, f[8:] * p
                    accs[2 * g] = a if tt == 0 else accs[2 * g] + a
                    accs[2 * g + 1] = b if tt == 0 else accs[2 * g + 1] + b
                hist.append(list(accs))
                if tt == nt - 1:
                    ab[slot][ps * gp * 16:(ps + 1) * gp * 16, :] = jnp.concatenate(accs, axis=0)
            mb[1 - slot][...] = st["mx"]
            lb[slot][...] = st["l"]

        def layer(li, x):
            first_layer = li == 0
            xn = _layernorm(x)
            xp = pltpu.bitcast(jnp.concatenate([xn, xn], axis=0).astype(BF16), U32)
            xn = xn.astype(BF16)
            q_proj(xn, 0, 0)
            q_proj(xn, 1, 1)

            @pl.when(first_layer)
            def _():
                wait(c_k[0] + c_vo[0])

            qf = qb[0][...].astype(BF16)
            mx = None
            for t in range(nt):
                s = qk_tile(qf, 0, t, 0)
                mx = s if mx is None else jnp.maximum(mx, s)
            mb[0][...] = mx
            yb[...] = jnp.zeros(yb.shape, F32)

            def body(it, carry):
                i0 = it * UNROLL

                @pl.when(first_layer)
                def _():
                    for c in range(1, nch):
                        @pl.when(i0 + UNROLL == starts[c])
                        def _():
                            wait(c_k[c])

                        @pl.when(i0 == starts[c])
                        def _():
                            wait(c_vo[c])

                for u in range(UNROLL):
                    if BARRIER:
                        @pl.when(one[u] > 0)
                        def _():
                            pair_step(xp, i0 + u, u % 2, u == 0)
                    else:
                        pair_step(xp, i0 + u, u % 2, u == 0)
                return carry

            lax.fori_loop(0, NP // UNROLL, body, 0)
            y = out_proj(yb[...], lb[(NP - 1) % 2][...], NP - 1, (NP - 1) % 2)
            x = x + jnp.sum(y, axis=0, keepdims=True)

            xn2 = _layernorm(x).astype(BF16)

            @pl.when(first_layer)
            def _():
                c_w1.wait()

            hid = jnp.dot(xn2, w1b[...], preferred_element_type=F32)
            hid = hid + b1b[...].astype(F32).reshape(1, FF)
            hid = jax.nn.gelu(hid, approximate=True).astype(BF16)
            x = x + b2b[...].astype(F32).reshape(1, D)
            for c in range(W2_CHUNKS):
                @pl.when(first_layer)
                def _():
                    c_w2[c].wait()

                x = x + jnp.dot(hid[:, c * f2:(c + 1) * f2], w2b[c * f2:(c + 1) * f2, :],
                                preferred_element_type=F32)
            return x

        wait(c_small + c_wq)
        x0 = jnp.broadcast_to(xb[...].astype(F32), (8, D))
        xf = lax.fori_loop(0, 2, layer, x0)
        o_ref[...] = xf[0:1].astype(o_ref.dtype)

    n_sems = 2 + 3 + 6 * nch + 1 + W2_CHUNKS
    return kernel, n_sems


@jax.jit
def pallas_interleave_layers__sliding_block_cached__dense_activation_gelu__decode_kernel(
    A_x: jax.Array,
    A_k_cache: jax.Array,
    A_v_cache: jax.Array,
    A_wq: jax.Array,
    A_wo: jax.Array,
    B_x: jax.Array,
    B_w1: jax.Array,
    B_b1: jax.Array,
    B_w2: jax.Array,
    B_b2: jax.Array,
):
    del B_x
    sk = A_k_cache.shape[2]
    win = min(4096, max(256, sk // 4))
    rows = H * DH
    kt = jnp.swapaxes(A_k_cache, 2, 3).reshape(rows // 16, 2, 8, sk)
    vt = jnp.swapaxes(A_v_cache, 2, 3).reshape(rows // 16, 2, 8, sk)
    wq = A_wq.reshape(D // 16, 2, 8, rows)
    wo = A_wo.reshape(rows // 16, 2, 8, D)
    kernel, n_sems = _make_kernel(sk, win)
    out = pl.pallas_call(
        kernel,
        out_shape=jax.ShapeDtypeStruct((1, D), A_x.dtype),
        in_specs=[pl.BlockSpec(memory_space=pl.ANY)] * 9,
        out_specs=pl.BlockSpec(memory_space=pltpu.VMEM),
        scratch_shapes=[
            pltpu.VMEM((rows // 16, 8, win), U32),
            pltpu.VMEM((rows // 16, 8, win), U32),
            pltpu.VMEM((D // 16, 8, rows), U32),
            pltpu.VMEM((rows // 16, 8, D), U32),
            pltpu.VMEM((D, FF), BF16),
            pltpu.VMEM((FF, D), BF16),
            pltpu.VMEM((1, D), BF16),
            pltpu.VMEM((FF,), BF16),
            pltpu.VMEM((D,), BF16),
            *[pltpu.VMEM((8, PW), F32)] * 2,
            *[pltpu.VMEM((8, win), F32)] * 2,
            *[pltpu.VMEM((8, win), F32)] * 2,
            *[pltpu.VMEM((PW, 128), F32)] * 2,
            *[pltpu.VMEM((8, 128), F32)] * 2,
            *[pltpu.VMEM((8, 128), F32)] * 2,
            pltpu.VMEM((8, 128), F32),
            pltpu.VMEM((8, D), F32),
            pltpu.SMEM((2 * UNROLL,), jnp.int32),
            pltpu.SemaphoreType.DMA((n_sems,)),
        ],
        compiler_params=pltpu.CompilerParams(vmem_limit_bytes=126 * 2**20),
        name="attn_ffn_decode",
    )(A_x.reshape(1, D), kt, vt, wq, wo, B_w1, B_b1, B_w2, B_b2)
    return out.reshape(A_x.shape)
```

```python
import numpy as np
import jax
import jax.numpy as jnp
from jax import lax
import jax.experimental.pallas as pl
import jax.experimental.pallas.tpu as pltpu

F32 = jnp.float32
BF16 = jnp.bfloat16
U32 = jnp.uint32

D = 640
H = 32
DH = 192
FF = 1536
NP = H // 2
PW = 2 * DH
G = PW // 16
NL = 2
W2_CHUNKS = 4

PASSES = 12
CHAIN = False
MAIN = (0, 4, 30, 32)
PENULT = (3, 0, 30, 48)
LAST = (12, 0, 30, 16)


def _bf(w):
    return pltpu.bitcast(w, BF16)


def _pack(v):
    return pltpu.bitcast(jnp.concatenate([v, v], axis=0).astype(BF16), U32)


def _mm(lhs, w):
    return jnp.dot(_bf(lhs), _bf(w), preferred_element_type=F32)[:8]


def _center(x):
    c = x - jnp.mean(x, axis=-1, keepdims=True)
    v = jnp.mean(c * c, axis=-1, keepdims=True)
    return c, 1.0 / jnp.sqrt(v + 1e-5)


def _tile(t):
    return slice(t * 128, (t + 1) * 128)


def _make_kernel(sk, win):
    nt = win // 128
    f2 = FF // W2_CHUNKS
    gp = G // PASSES
    exp_scale = np.float32(DH ** -0.5 * np.log2(np.e))

    def kernel(x_hbm, k_hbm, v_hbm, wq_hbm, wo_hbm, w1_hbm, b1_hbm, w2_hbm, b2_hbm,
               o_ref,
               kbuf, vbuf, wqb, wob, w1b, w2b, xb, b1b, b2b,
               q0, q1, sb, p0, p1, a0, a1, e0, e1, lp, lc, zb, yb, one, sems):
        qb, pb, ab, eb = (q0, q1), (p0, p1), (a0, a1), (e0, e1)

        copies = []

        def copy(src, dst):
            copies.append(pltpu.make_async_copy(src, dst, sems.at[len(copies)]))
            return [copies[-1]]

        def halves(src, dst, g0, g1, cols):
            s = src.bitcast(U32)
            rows = pl.ds(g0, g1 - g0)
            return (copy(s.at[rows, 0, :, cols], dst.at[rows, pl.ds(0, 4), :])
                    + copy(s.at[rows, 1, :, cols], dst.at[rows, pl.ds(4, 4), :]))

        window = pl.ds(sk - win, win)
        c_head = (halves(k_hbm, kbuf, 0, (NP - 1) * G, window)
                  + halves(v_hbm, vbuf, 0, (NP - 2) * G, window)
                  + halves(wq_hbm, wqb, 0, D // 16, pl.ds(0, H * DH))
                  + halves(wo_hbm, wob, 0, (NP - 3) * G, pl.ds(0, D))
                  + copy(x_hbm, xb) + copy(b1_hbm, b1b) + copy(b2_hbm, b2b))
        c_tail = (halves(k_hbm, kbuf, (NP - 1) * G, NP * G, window)
                  + halves(v_hbm, vbuf, (NP - 2) * G, NP * G, window)
                  + halves(wo_hbm, wob, (NP - 3) * G, NP * G, pl.ds(0, D)))
        c_w1 = copy(w1_hbm, w1b)
        c_w2 = [copy(w2_hbm.at[pl.ds(i * f2, f2)], w2b.at[pl.ds(i * f2, f2)])
                for i in range(W2_CHUNKS)]
        for c in copies:
            c.start()

        def wait(cs):
            for c in cs:
                c.wait()

        zb[...] = jnp.zeros(zb.shape, F32)
        a1[...] = jnp.zeros(a1.shape, F32)
        e0[...] = jnp.zeros(e0.shape, F32)
        e1[...] = jnp.zeros(e1.shape, F32)
        lp[...] = jnp.ones(lp.shape, F32)
        for u in range(4):
            one[u] = 1

        row = lax.broadcasted_iota(jnp.int32, (8, PW), 0)
        lane = lax.broadcasted_iota(jnp.int32, (8, PW), 1)
        bd = ((row == 0) & (lane < DH)) | ((row == 1) & (lane >= DH))

        def q_tile(xc, rs, j, c, slot):
            start = j * PW + c * 128
            if not isinstance(start, int):
                start = pl.multiple_of(start, 128)
            q = _mm(xc, wqb[:, :, pl.ds(start, 128)].reshape(D // 2, 128)) * rs
            qb[slot][:, _tile(c)] = jnp.where(bd[:, _tile(c)], q, 0.0)

        def qk_tile(q, j, t):
            s = _mm(q, kbuf[pl.ds(j * G, G), :, _tile(t)].reshape(PW // 2, 128))
            sb[:, _tile(t)] = s
            return s

        def exp_tile(m, t, slot):
            p = jnp.exp2((sb[:, _tile(t)] - m) * exp_scale)
            pb[slot][:, _tile(t)] = p
            return p

        def key_sum(a):
            a = jnp.sum(a.T.reshape(16, 8, 128), axis=0)
            return jnp.broadcast_to(jnp.sum(a, axis=0, keepdims=True), (8, 128))

        def normalize(cols, l, slot, mask):
            o = jnp.concatenate(cols, axis=1) + eb[slot][...]
            return _pack(jnp.where(mask, o / jnp.sum(l, axis=-1, keepdims=True), 0.0))

        def out_tile(o, j, c):
            return _mm(o, wob[pl.ds(j * G, G), :, _tile(c)].reshape(PW // 2, 128))

        def pair_step(xc, rs, i, slot, cfg, do_qk, do_q, maybe_first):
            mxu_tiles, gate, tail, tstep = cfg
            nv = nt - mxu_tiles
            ns = PASSES * nv
            flag = zb[...] > 0.0
            l_prev = lp[...]
            lp[...] = lc[...]
            hist = []
            st = dict(n=0, l=None, mx=None, cols=[])
            if do_qk:
                st["q"] = _pack(qb[1 - slot][...])

            def gated(v, pos):
                if pos <= gate:
                    return v
                st["n"] += 1
                a = hist[pos - 1 - gate][st["n"] % (2 * gp)]
                g = jnp.where(flag, pltpu.bitcast(a, v.dtype), v[:8, :128])
                if v.shape[1] > 128:
                    return jnp.concatenate([g, v[:, 128:]], axis=1)
                return g if v.shape[0] == 8 else jnp.concatenate([g, v[8:]], axis=0)

            def job_qk(t, pos):
                s = qk_tile(gated(st["q"], pos), i + 1, t)
                st["mx"] = s if t == 0 else jnp.maximum(st["mx"], s)

            def job_exp(t, pos):
                if t == 0:
                    st["m"] = jnp.max(st["mx"], axis=-1, keepdims=True)
                p = exp_tile(st["m"], t, 1 - slot)
                st["l"] = p if t == 0 else st["l"] + p
                if t == nt - 1:
                    lc[...] = st["l"]

            def job_q(c, pos):
                q_tile(gated(xc, pos), rs, i + 2, c, slot)

            def job_t(c, pos):
                st["cols"].append(key_sum(gated(ab[1 - slot][_tile(c), :], pos)))
                if c == PW // 128 - 1:
                    mask = bd & (i > 0) if maybe_first else bd
                    st["o"] = normalize(st["cols"], l_prev, 1 - slot, mask)

            def job_o(c, pos):
                j = jnp.maximum(i - 1, 0) if maybe_first else i - 1
                yb[:, _tile(c)] += out_tile(gated(st["o"], pos), j, c)

            def job_pv(t, pos):
                lhs = _bf(gated(_pack(pb[slot][:, _tile(t)]), pos))
                w = _bf(vbuf[pl.ds(i * G, G), :, _tile(t)].reshape(PW // 2, 128))
                e = lax.dot_general(lhs, w, (((1,), (1,)), ((), ())),
                                    preferred_element_type=F32)[:8]
                st["e"] = e if t == nv else st["e"] + e
                if t == nt - 1:
                    eb[slot][...] = st["e"]

            qk = [(job_qk, t, 3) for t in range(nt)] if do_qk else []
            out = [(job_o, c, 3) for c in range(D // 128)]
            pv = [(job_pv, t, 6) for t in range(nv, nt)]
            qp = [(job_q, c, 5) for c in range(PW // 128)] if do_q else []
            jobs = qk + out + pv + qp if do_qk else pv + out
            total = sum(j[2] for j in jobs)
            at, done = {}, 0
            for c in range(PW // 128):
                at.setdefault(c * tstep, []).append((job_t, c))
            for fn, arg, cost in jobs:
                at.setdefault(done * (ns - tail) // total, []).append((fn, arg))
                done += cost
            if do_qk:
                for t in range(nt):
                    at.setdefault(ns - nt + t, []).append((job_exp, t))

            accs = None
            for pos in range(ns):
                ps, tt = divmod(pos, nv)
                for fn, arg in at.get(pos, []):
                    fn(arg, pos)
                h = ps * 2 // PASSES
                p = jnp.broadcast_to(pb[slot][pl.ds(h, 1), _tile(tt)], (8, 128))
                if CHAIN and tt == 0 and ps > 0:
                    p = jnp.where(flag, accs[0], p)
                new = []
                for g in range(gp):
                    f = _bf(vbuf[i * G + ps * gp + g, :, _tile(tt)]).astype(F32)
                    new += [f[:8] * p, f[8:] * p]
                accs = new if tt == 0 else [a + b for a, b in zip(accs, new)]
                hist.append(accs)
                if tt == nv - 1:
                    ab[slot][ps * gp * 16:(ps + 1) * gp * 16, :] = jnp.concatenate(accs, axis=0)

        def finish(x, dma):
            slot = (NP - 1) % 2
            cols = [key_sum(ab[slot][_tile(c), :]) for c in range(PW // 128)]
            o = normalize(cols, lp[...], slot, bd)
            y = jnp.concatenate([out_tile(o, NP - 1, c) for c in range(D // 128)], axis=1)
            x = x + jnp.sum(yb[...] + y, axis=0, keepdims=True)
            if MAIN[0] == 0:
                e0[...] = jnp.zeros(e0.shape, F32)
                e1[...] = jnp.zeros(e1.shape, F32)
            xc, rs = _center(x)
            if dma:
                wait(c_w1)
            hid = jnp.dot(xc.astype(BF16), w1b[...], preferred_element_type=F32) * rs
            hid = hid + b1b[...].astype(F32).reshape(1, FF)
            hid = jax.nn.gelu(hid, approximate=True).astype(BF16)
            x = x + b2b[...].astype(F32).reshape(1, D)
            for c in range(W2_CHUNKS):
                if dma:
                    wait(c_w2[c])
                x = x + jnp.dot(hid[:, c * f2:(c + 1) * f2], w2b[c * f2:(c + 1) * f2, :],
                                preferred_element_type=F32)
            return x

        def layer(li, x):
            xc, rs = _center(x)
            xc = _pack(xc)
            for c in range(PW // 128):
                q_tile(xc, rs, 0, c, 0)
            q = _pack(q0[...])
            mx = None
            for t in range(nt):
                s = qk_tile(q, 0, t)
                mx = s if t == 0 else jnp.maximum(mx, s)
            for c in range(PW // 128):
                q_tile(xc, rs, 1, c, 1)
            m = jnp.max(mx, axis=-1, keepdims=True)
            lc[...] = sum(exp_tile(m, t, 0) for t in range(nt))
            yb[...] = jnp.zeros(yb.shape, F32)

            def body(it, carry):
                for u in range(2):
                    @pl.when(one[u] > 0)
                    def _():
                        pair_step(xc, rs, 2 * it + u, u, MAIN, True, True, u == 0)
                return carry

            lax.fori_loop(0, NP // 2 - 1, body, 0)

            @pl.when(li == 0)
            def _():
                wait(c_tail)

            @pl.when(one[2] > 0)
            def _():
                pair_step(xc, rs, NP - 2, 0, PENULT, True, False, False)

            @pl.when(one[3] > 0)
            def _():
                pair_step(xc, rs, NP - 1, 1, LAST, False, False, False)

            return lax.cond(li == 0, lambda: finish(x, True), lambda: finish(x, False))

        wait(c_head)
        x0 = jnp.broadcast_to(xb[...].astype(F32), (8, D))
        o_ref[...] = lax.fori_loop(0, NL, layer, x0)[0:1].astype(o_ref.dtype)

    return kernel, 18 + W2_CHUNKS


@jax.jit
def pallas_interleave_layers__sliding_block_cached__dense_activation_gelu__decode_kernel(
    A_x: jax.Array,
    A_k_cache: jax.Array,
    A_v_cache: jax.Array,
    A_wq: jax.Array,
    A_wo: jax.Array,
    B_x: jax.Array,
    B_w1: jax.Array,
    B_b1: jax.Array,
    B_w2: jax.Array,
    B_b2: jax.Array,
):
    del B_x
    sk = A_k_cache.shape[2]
    win = min(4096, max(256, sk // 4))
    rows = H * DH
    kt = jnp.swapaxes(A_k_cache, 2, 3).reshape(rows // 16, 2, 8, sk)
    vt = jnp.swapaxes(A_v_cache, 2, 3).reshape(rows // 16, 2, 8, sk)
    wq = A_wq.reshape(D // 16, 2, 8, rows)
    wo = A_wo.reshape(rows // 16, 2, 8, D)
    kernel, n_sems = _make_kernel(sk, win)
    out = pl.pallas_call(
        kernel,
        out_shape=jax.ShapeDtypeStruct((1, D), A_x.dtype),
        in_specs=[pl.BlockSpec(memory_space=pl.ANY)] * 9,
        out_specs=pl.BlockSpec(memory_space=pltpu.VMEM),
        scratch_shapes=[
            pltpu.VMEM((rows // 16, 8, win), U32),
            pltpu.VMEM((rows // 16, 8, win), U32),
            pltpu.VMEM((D // 16, 8, rows), U32),
            pltpu.VMEM((rows // 16, 8, D), U32),
            pltpu.VMEM((D, FF), BF16),
            pltpu.VMEM((FF, D), BF16),
            pltpu.VMEM((1, D), BF16),
            pltpu.VMEM((FF,), BF16),
            pltpu.VMEM((D,), BF16),
            *[pltpu.VMEM((8, PW), F32)] * 2,
            pltpu.VMEM((8, win), F32),
            *[pltpu.VMEM((8, win), F32)] * 2,
            *[pltpu.VMEM((PW, 128), F32)] * 2,
            *[pltpu.VMEM((8, PW), F32)] * 2,
            *[pltpu.VMEM((8, 128), F32)] * 2,
            pltpu.VMEM((8, 128), F32),
            pltpu.VMEM((8, D), F32),
            pltpu.SMEM((4,), jnp.int32),
            pltpu.SemaphoreType.DMA((n_sems,)),
        ],
        compiler_params=pltpu.CompilerParams(vmem_limit_bytes=126 * 2**20),
        name="attn_ffn_decode",
    )(A_x.reshape(1, D), kt, vt, wq, wo, B_w1, B_b1, B_w2, B_b2)
    return out.reshape(A_x.shape)
```

```python
import numpy as np
import jax
import jax.numpy as jnp
from jax import lax
import jax.experimental.pallas as pl
import jax.experimental.pallas.tpu as pltpu

F32 = jnp.float32
BF16 = jnp.bfloat16
U32 = jnp.uint32

D = 640
H = 32
DH = 192
FF = 1536
NP = H // 2
PW = 2 * DH
G = PW // 16
NL = 2
W2_CHUNKS = 4

PASSES = 12
CHAIN = False
MAIN = (0, 4, 30, 32)
PENULT = (3, 0, 30, 48)
LAST = (12, 0, 30, 16)


def _bf(w):
    return pltpu.bitcast(w, BF16)


def _pack(v):
    return pltpu.bitcast(jnp.concatenate([v, v], axis=0).astype(BF16), U32)


def _mm(lhs, w):
    return jnp.dot(_bf(lhs), _bf(w), preferred_element_type=F32)[:8]


def _center(x):
    c = x - jnp.mean(x, axis=-1, keepdims=True)
    v = jnp.mean(c * c, axis=-1, keepdims=True)
    return c, 1.0 / jnp.sqrt(v + 1e-5)


def _tile(t):
    return slice(t * 128, (t + 1) * 128)


def _make_kernel(sk, win):
    nt = win // 128
    f2 = FF // W2_CHUNKS
    gp = G // PASSES
    exp_scale = np.float32(DH ** -0.5 * np.log2(np.e))

    def kernel(x_hbm, k_hbm, v_hbm, wq_hbm, wo_hbm, w1_hbm, b1_hbm, w2_hbm, b2_hbm,
               o_ref,
               kbuf, vbuf, wqb, wob, w1b, w2b, xb, b1b, b2b,
               q0, q1, sb, p0, p1, a0, a1, e0, e1, lp, lc, zb, yb, one, sems):
        qb, pb, ab, eb = (q0, q1), (p0, p1), (a0, a1), (e0, e1)

        copies = []

        def copy(src, dst):
            copies.append(pltpu.make_async_copy(src, dst, sems.at[len(copies)]))
            return [copies[-1]]

        def halves(src, dst, g0, g1, cols):
            s = src.bitcast(U32)
            rows = pl.ds(g0, g1 - g0)
            return (copy(s.at[rows, 0, :, cols], dst.at[rows, pl.ds(0, 4), :])
                    + copy(s.at[rows, 1, :, cols], dst.at[rows, pl.ds(4, 4), :]))

        window = pl.ds(sk - win, win)
        c_head = (halves(k_hbm, kbuf, 0, (NP - 1) * G, window)
                  + halves(v_hbm, vbuf, 0, (NP - 2) * G, window)
                  + halves(wq_hbm, wqb, 0, D // 16, pl.ds(0, H * DH))
                  + halves(wo_hbm, wob, 0, (NP - 3) * G, pl.ds(0, D))
                  + copy(x_hbm, xb) + copy(b1_hbm, b1b) + copy(b2_hbm, b2b))
        c_tail = (halves(k_hbm, kbuf, (NP - 1) * G, NP * G, window)
                  + halves(v_hbm, vbuf, (NP - 2) * G, NP * G, window)
                  + halves(wo_hbm, wob, (NP - 3) * G, NP * G, pl.ds(0, D)))
        c_w1 = copy(w1_hbm, w1b)
        c_w2 = [copy(w2_hbm.at[pl.ds(i * f2, f2)], w2b.at[pl.ds(i * f2, f2)])
                for i in range(W2_CHUNKS)]
        for c in copies:
            c.start()

        def wait(cs):
            for c in cs:
                c.wait()

        zb[...] = jnp.zeros(zb.shape, F32)
        a1[...] = jnp.zeros(a1.shape, F32)
        e0[...] = jnp.zeros(e0.shape, F32)
        e1[...] = jnp.zeros(e1.shape, F32)
        lp[...] = jnp.ones(lp.shape, F32)
        for u in range(4):
            one[u] = 1

        row = lax.broadcasted_iota(jnp.int32, (8, PW), 0)
        lane = lax.broadcasted_iota(jnp.int32, (8, PW), 1)
        bd = ((row == 0) & (lane < DH)) | ((row == 1) & (lane >= DH))

        def q_tile(xc, rs, j, c, slot):
            start = j * PW + c * 128
            if not isinstance(start, int):
                start = pl.multiple_of(start, 128)
            q = _mm(xc, wqb[:, :, pl.ds(start, 128)].reshape(D // 2, 128)) * rs
            qb[slot][:, _tile(c)] = jnp.where(bd[:, _tile(c)], q, 0.0)

        def qk_tile(q, j, t):
            s = _mm(q, kbuf[pl.ds(j * G, G), :, _tile(t)].reshape(PW // 2, 128))
            sb[:, _tile(t)] = s
            return s

        def exp_tile(m, t, slot):
            p = jnp.exp2(sb[:, _tile(t)] - m)
            pb[slot][:, _tile(t)] = p
            return p

        def key_sum(a):
            a = jnp.sum(a.T.reshape(16, 8, 128), axis=0)
            return jnp.broadcast_to(jnp.sum(a, axis=0, keepdims=True), (8, 128))

        def normalize(cols, l, slot, mask):
            o = jnp.concatenate(cols, axis=1) + eb[slot][...]
            return _pack(jnp.where(mask, o / jnp.sum(l, axis=-1, keepdims=True), 0.0))

        def out_tile(o, j, c):
            return _mm(o, wob[pl.ds(j * G, G), :, _tile(c)].reshape(PW // 2, 128))

        def pair_step(xc, rs, i, slot, cfg, do_qk, do_q, maybe_first):
            mxu_tiles, gate, tail, tstep = cfg
            nv = nt - mxu_tiles
            ns = PASSES * nv
            flag = zb[...] > 0.0
            l_prev = lp[...]
            lp[...] = lc[...]
            hist = []
            st = dict(n=0, l=None, mx=None, cols=[])
            if do_qk:
                st["q"] = _pack(qb[1 - slot][...])

            def gated(v, pos):
                if pos <= gate:
                    return v
                st["n"] += 1
                a = hist[pos - 1 - gate][st["n"] % (2 * gp)]
                g = jnp.where(flag, pltpu.bitcast(a, v.dtype), v[:8, :128])
                if v.shape[1] > 128:
                    return jnp.concatenate([g, v[:, 128:]], axis=1)
                return g if v.shape[0] == 8 else jnp.concatenate([g, v[8:]], axis=0)

            def job_qk(t, pos):
                s = qk_tile(gated(st["q"], pos), i + 1, t)
                st["mx"] = s if t == 0 else jnp.maximum(st["mx"], s)

            def job_exp(t, pos):
                if t == 0:
                    st["m"] = jnp.max(st["mx"], axis=-1, keepdims=True)
                p = exp_tile(st["m"], t, 1 - slot)
                st["l"] = p if t == 0 else st["l"] + p
                if t == nt - 1:
                    lc[...] = st["l"]

            def job_q(c, pos):
                q_tile(gated(xc, pos), rs, i + 2, c, slot)

            def job_t(c, pos):
                st["cols"].append(key_sum(gated(ab[1 - slot][_tile(c), :], pos)))
                if c == PW // 128 - 1:
                    mask = bd & (i > 0) if maybe_first else bd
                    st["o"] = normalize(st["cols"], l_prev, 1 - slot, mask)

            def job_o(c, pos):
                j = jnp.maximum(i - 1, 0) if maybe_first else i - 1
                yb[:, _tile(c)] += out_tile(gated(st["o"], pos), j, c)

            def job_pv(t, pos):
                lhs = _bf(gated(_pack(pb[slot][:, _tile(t)]), pos))
                w = _bf(vbuf[pl.ds(i * G, G), :, _tile(t)].reshape(PW // 2, 128))
                e = lax.dot_general(lhs, w, (((1,), (1,)), ((), ())),
                                    preferred_element_type=F32)[:8]
                st["e"] = e if t == nv else st["e"] + e
                if t == nt - 1:
                    eb[slot][...] = st["e"]

            qk = [(job_qk, t, 3) for t in range(nt)] if do_qk else []
            out = [(job_o, c, 3) for c in range(D // 128)]
            pv = [(job_pv, t, 6) for t in range(nv, nt)]
            qp = [(job_q, c, 5) for c in range(PW // 128)] if do_q else []
            jobs = qk + out + pv + qp if do_qk else pv + out
            total = sum(j[2] for j in jobs)
            at, done = {}, 0
            for c in range(PW // 128):
                at.setdefault(c * tstep, []).append((job_t, c))
            for fn, arg, cost in jobs:
                at.setdefault(done * (ns - tail) // total, []).append((fn, arg))
                done += cost
            if do_qk:
                for t in range(nt):
                    at.setdefault(ns - nt + t, []).append((job_exp, t))

            accs = None
            for pos in range(ns):
                ps, tt = divmod(pos, nv)
                for fn, arg in at.get(pos, []):
                    fn(arg, pos)
                h = ps * 2 // PASSES
                p = jnp.broadcast_to(pb[slot][pl.ds(h, 1), _tile(tt)], (8, 128))
                if CHAIN and tt == 0 and ps > 0:
                    p = jnp.where(flag, accs[0], p)
                new = []
                for g in range(gp):
                    f = _bf(vbuf[i * G + ps * gp + g, :, _tile(tt)]).astype(F32)
                    new += [f[:8] * p, f[8:] * p]
                accs = new if tt == 0 else [a + b for a, b in zip(accs, new)]
                hist.append(accs)
                if tt == nv - 1:
                    ab[slot][ps * gp * 16:(ps + 1) * gp * 16, :] = jnp.concatenate(accs, axis=0)

        def finish(x, dma):
            slot = (NP - 1) % 2
            cols = [key_sum(ab[slot][_tile(c), :]) for c in range(PW // 128)]
            o = normalize(cols, lp[...], slot, bd)
            y = jnp.concatenate([out_tile(o, NP - 1, c) for c in range(D // 128)], axis=1)
            x = x + jnp.sum(yb[...] + y, axis=0, keepdims=True)
            if MAIN[0] == 0:
                e0[...] = jnp.zeros(e0.shape, F32)
                e1[...] = jnp.zeros(e1.shape, F32)
            xc, rs = _center(x)
            if dma:
                wait(c_w1)
            hid = jnp.dot(xc.astype(BF16), w1b[...], preferred_element_type=F32) * rs
            hid = hid + b1b[...].astype(F32).reshape(1, FF)
            hid = jax.nn.gelu(hid, approximate=True).astype(BF16)
            x = x + b2b[...].astype(F32).reshape(1, D)
            for c in range(W2_CHUNKS):
                if dma:
                    wait(c_w2[c])
                x = x + jnp.dot(hid[:, c * f2:(c + 1) * f2], w2b[c * f2:(c + 1) * f2, :],
                                preferred_element_type=F32)
            return x

        def layer(li, x):
            xc, rs = _center(x)
            xc, rs = _pack(xc), rs * exp_scale
            for c in range(PW // 128):
                q_tile(xc, rs, 0, c, 0)
            q = _pack(q0[...])
            mx = None
            for t in range(nt):
                s = qk_tile(q, 0, t)
                mx = s if t == 0 else jnp.maximum(mx, s)
            for c in range(PW // 128):
                q_tile(xc, rs, 1, c, 1)
            m = jnp.max(mx, axis=-1, keepdims=True)
            lc[...] = sum(exp_tile(m, t, 0) for t in range(nt))
            yb[...] = jnp.zeros(yb.shape, F32)

            def body(it, carry):
                for u in range(2):
                    @pl.when(one[u] > 0)
                    def _():
                        pair_step(xc, rs, 2 * it + u, u, MAIN, True, True, u == 0)
                return carry

            lax.fori_loop(0, NP // 2 - 1, body, 0)

            @pl.when(li == 0)
            def _():
                wait(c_tail)

            @pl.when(one[2] > 0)
            def _():
                pair_step(xc, rs, NP - 2, 0, PENULT, True, False, False)

            @pl.when(one[3] > 0)
            def _():
                pair_step(xc, rs, NP - 1, 1, LAST, False, False, False)

            return lax.cond(li == 0, lambda: finish(x, True), lambda: finish(x, False))

        wait(c_head)
        if NL == 0:
            wait(copies[len(c_head):])
        x0 = jnp.broadcast_to(xb[...].astype(F32), (8, D))
        o_ref[...] = lax.fori_loop(0, NL, layer, x0)[0:1].astype(o_ref.dtype)

    return kernel, 18 + W2_CHUNKS


@jax.jit
def pallas_interleave_layers__sliding_block_cached__dense_activation_gelu__decode_kernel(
    A_x: jax.Array,
    A_k_cache: jax.Array,
    A_v_cache: jax.Array,
    A_wq: jax.Array,
    A_wo: jax.Array,
    B_x: jax.Array,
    B_w1: jax.Array,
    B_b1: jax.Array,
    B_w2: jax.Array,
    B_b2: jax.Array,
):
    del B_x
    sk = A_k_cache.shape[2]
    win = min(4096, max(256, sk // 4))
    rows = H * DH
    kt = jnp.swapaxes(A_k_cache, 2, 3).reshape(rows // 16, 2, 8, sk)
    vt = jnp.swapaxes(A_v_cache, 2, 3).reshape(rows // 16, 2, 8, sk)
    wq = A_wq.reshape(D // 16, 2, 8, rows)
    wo = A_wo.reshape(rows // 16, 2, 8, D)
    kernel, n_sems = _make_kernel(sk, win)
    out = pl.pallas_call(
        kernel,
        out_shape=jax.ShapeDtypeStruct((1, D), A_x.dtype),
        in_specs=[pl.BlockSpec(memory_space=pl.ANY)] * 9,
        out_specs=pl.BlockSpec(memory_space=pltpu.VMEM),
        scratch_shapes=[
            pltpu.VMEM((rows // 16, 8, win), U32),
            pltpu.VMEM((rows // 16, 8, win), U32),
            pltpu.VMEM((D // 16, 8, rows), U32),
            pltpu.VMEM((rows // 16, 8, D), U32),
            pltpu.VMEM((D, FF), BF16),
            pltpu.VMEM((FF, D), BF16),
            pltpu.VMEM((1, D), BF16),
            pltpu.VMEM((FF,), BF16),
            pltpu.VMEM((D,), BF16),
            *[pltpu.VMEM((8, PW), F32)] * 2,
            pltpu.VMEM((8, win), F32),
            *[pltpu.VMEM((8, win), F32)] * 2,
            *[pltpu.VMEM((PW, 128), F32)] * 2,
            *[pltpu.VMEM((8, PW), F32)] * 2,
            *[pltpu.VMEM((8, 128), F32)] * 2,
            pltpu.VMEM((8, 128), F32),
            pltpu.VMEM((8, D), F32),
            pltpu.SMEM((4,), jnp.int32),
            pltpu.SemaphoreType.DMA((n_sems,)),
        ],
        compiler_params=pltpu.CompilerParams(vmem_limit_bytes=126 * 2**20),
        name="attn_ffn_decode",
    )(A_x.reshape(1, D), kt, vt, wq, wo, B_w1, B_b1, B_w2, B_b2)
    return out.reshape(A_x.shape)
```

```python
import numpy as np
import jax
import jax.numpy as jnp
from jax import lax
import jax.experimental.pallas as pl
import jax.experimental.pallas.tpu as pltpu

F32 = jnp.float32
BF16 = jnp.bfloat16
U32 = jnp.uint32

D = 640
H = 32
DH = 192
FF = 1536
NP = H // 2
PW = 2 * DH
G = PW // 16
NL = 2
W2_CHUNKS = 4

PASSES = 12
CHAIN = False
PVJ = 4
PVFIRST = False
MAIN = (3, 4, 30, 32)
PENULT = (5, 0, 30, 48)
LAST = (18, 0, 30, 16)


def _bf(w):
    return pltpu.bitcast(w, BF16)


def _pack(v):
    return pltpu.bitcast(jnp.concatenate([v, v], axis=0).astype(BF16), U32)


def _mm(lhs, w):
    return jnp.dot(_bf(lhs), _bf(w), preferred_element_type=F32)[:8]


def _center(x):
    c = x - jnp.mean(x, axis=-1, keepdims=True)
    v = jnp.mean(c * c, axis=-1, keepdims=True)
    return c, 1.0 / jnp.sqrt(v + 1e-5)


def _tile(t):
    return slice(t * 128, (t + 1) * 128)


def _make_kernel(sk, win):
    nt = win // 128
    f2 = FF // W2_CHUNKS
    gp = G // PASSES
    exp_scale = np.float32(DH ** -0.5 * np.log2(np.e))

    def kernel(x_hbm, k_hbm, v_hbm, wq_hbm, wo_hbm, w1_hbm, b1_hbm, w2_hbm, b2_hbm,
               o_ref,
               kbuf, vbuf, wqb, wob, w1b, w2b, xb, b1b, b2b,
               vt_main, vt_pen, vt_last, q0, q1, sb, p0, p1, a0, a1, e0, e1, lp, lc, zb, yb, one, sems):
        qb, pb, ab, eb = (q0, q1), (p0, p1), (a0, a1), (e0, e1)

        copies = []

        def copy(src, dst):
            copies.append(pltpu.make_async_copy(src, dst, sems.at[len(copies)]))
            return [copies[-1]]

        def halves(src, dst, g0, g1, cols):
            s = src.bitcast(U32)
            rows = pl.ds(g0, g1 - g0)
            return (copy(s.at[rows, 0, :, cols], dst.at[rows, pl.ds(0, 4), :])
                    + copy(s.at[rows, 1, :, cols], dst.at[rows, pl.ds(4, 4), :]))

        window = pl.ds(sk - win, win)
        c_v0 = halves(v_hbm, vbuf, 0, (NP - 2) * G, window)
        c_head = (halves(k_hbm, kbuf, 0, (NP - 1) * G, window)
                  + halves(wq_hbm, wqb, 0, D // 16, pl.ds(0, H * DH))
                  + halves(wo_hbm, wob, 0, (NP - 3) * G, pl.ds(0, D))
                  + copy(x_hbm, xb) + copy(b1_hbm, b1b) + copy(b2_hbm, b2b))
        c_v1 = halves(v_hbm, vbuf, (NP - 2) * G, NP * G, window)
        c_tail = (halves(k_hbm, kbuf, (NP - 1) * G, NP * G, window)
                  + halves(wo_hbm, wob, (NP - 3) * G, NP * G, pl.ds(0, D)))
        c_w1 = copy(w1_hbm, w1b)
        c_w2 = [copy(w2_hbm.at[pl.ds(i * f2, f2)], w2b.at[pl.ds(i * f2, f2)])
                for i in range(W2_CHUNKS)]
        for c in copies:
            c.start()

        def wait(cs):
            for c in cs:
                c.wait()

        zb[...] = jnp.zeros(zb.shape, F32)
        a1[...] = jnp.zeros(a1.shape, F32)
        e1[...] = jnp.zeros(e1.shape, F32)
        lp[...] = jnp.ones(lp.shape, F32)
        for u in range(4):
            one[u] = 1

        row = lax.broadcasted_iota(jnp.int32, (8, PW), 0)
        lane = lax.broadcasted_iota(jnp.int32, (8, PW), 1)
        bd = ((row == 0) & (lane < DH)) | ((row == 1) & (lane >= DH))

        def q_tile(xc, rs, j, c, slot):
            start = j * PW + c * 128
            if not isinstance(start, int):
                start = pl.multiple_of(start, 128)
            q = _mm(xc, wqb[:, :, pl.ds(start, 128)].reshape(D // 2, 128)) * rs
            qb[slot][:, _tile(c)] = jnp.where(bd[:, _tile(c)], q, 0.0)

        def qk_tile(q, j, t):
            s = _mm(q, kbuf[pl.ds(j * G, G), :, _tile(t)].reshape(PW // 2, 128))
            sb[:, _tile(t)] = s
            return s

        def exp_tile(m, t, slot):
            p = jnp.exp2(sb[:, _tile(t)] - m)
            pb[slot][:, _tile(t)] = p
            return p

        def key_sum(a):
            a = jnp.sum(a.T.reshape(16, 8, 128), axis=0)
            return jnp.broadcast_to(jnp.sum(a, axis=0, keepdims=True), (8, 128))

        def normalize(cols, l, slot, mask):
            o = jnp.concatenate(cols, axis=1) + eb[slot][...]
            return _pack(jnp.where(mask, o / jnp.sum(l, axis=-1, keepdims=True), 0.0))

        def out_tile(o, j, c):
            return _mm(o, wob[pl.ds(j * G, G), :, _tile(c)].reshape(PW // 2, 128))

        def transpose_v(j, vt, n):
            for t in range(n):
                w = _bf(vbuf[pl.ds(j * G, G), :, _tile(nt - n + t)].reshape(PW // 2, 128))
                vt[t * 64:(t + 1) * 64, :] = pltpu.bitcast(w.T, U32)

        def pair_step(xc, rs, i, slot, cfg, vt, do_qk, do_q, maybe_first):
            mxu_tiles, gate, tail, tstep = cfg
            nv = nt - mxu_tiles
            ns = PASSES * nv
            flag = zb[...] > 0.0
            l_prev = lp[...]
            lp[...] = lc[...]
            hist = []
            st = dict(n=0, l=None, mx=None, cols=[])
            if do_qk:
                st["q"] = _pack(qb[1 - slot][...])

            def gated(v, pos):
                if pos <= gate:
                    return v
                st["n"] += 1
                a = hist[pos - 1 - gate][st["n"] % (2 * gp)]
                g = jnp.where(flag, pltpu.bitcast(a, v.dtype), v[:8, :128])
                if v.shape[1] > 128:
                    return jnp.concatenate([g, v[:, 128:]], axis=1)
                return g if v.shape[0] == 8 else jnp.concatenate([g, v[8:]], axis=0)

            def job_qk(t, pos):
                s = qk_tile(gated(st["q"], pos), i + 1, t)
                st["mx"] = s if t == 0 else jnp.maximum(st["mx"], s)

            def job_exp(t, pos):
                if t == 0:
                    st["m"] = jnp.max(st["mx"], axis=-1, keepdims=True)
                p = exp_tile(st["m"], t, 1 - slot)
                st["l"] = p if t == 0 else st["l"] + p
                if t == nt - 1:
                    lc[...] = st["l"]

            def job_q(c, pos):
                q_tile(gated(xc, pos), rs, i + 2, c, slot)

            def job_t(c, pos):
                st["cols"].append(key_sum(gated(ab[1 - slot][_tile(c), :], pos)))
                if c == PW // 128 - 1:
                    mask = bd & (i > 0) if maybe_first else bd
                    st["o"] = normalize(st["cols"], l_prev, 1 - slot, mask)

            def job_o(c, pos):
                j = jnp.maximum(i - 1, 0) if maybe_first else i - 1
                yb[:, _tile(c)] += out_tile(gated(st["o"], pos), j, c)

            def job_pv(arg, pos):
                c, t0, t1 = arg
                lhs = _pack(pb[slot][:, (nv + t0) * 128:(nv + t1) * 128])
                e = _mm(gated(lhs, pos), vt[t0 * 64:t1 * 64, _tile(c)])
                st["e"] = e if t0 == 0 else st["e"] + e
                if t1 == mxu_tiles:
                    eb[slot][:, _tile(c)] = st["e"]

            qk = [(job_qk, t, 3) for t in range(nt)] if do_qk else []
            out = [(job_o, c, 3) for c in range(D // 128)]
            pv = [(job_pv, (c, t, min(t + PVJ, mxu_tiles)), min(PVJ, mxu_tiles - t))
                  for c in range(PW // 128) for t in range(0, mxu_tiles, PVJ)]
            qp = [(job_q, c, 5) for c in range(PW // 128)] if do_q else []
            jobs = (pv + qk + out + qp if PVFIRST else qk + pv + out + qp)
            total = sum(j[2] for j in jobs)
            at, done = {}, 0
            for c in range(PW // 128):
                at.setdefault(c * tstep, []).append((job_t, c))
            for fn, arg, cost in jobs:
                at.setdefault(done * (ns - tail) // total, []).append((fn, arg))
                done += cost
            if do_qk:
                for t in range(nt):
                    at.setdefault(ns - nt + t, []).append((job_exp, t))

            accs = None
            for pos in range(ns):
                ps, tt = divmod(pos, nv)
                for fn, arg in at.get(pos, []):
                    fn(arg, pos)
                h = ps * 2 // PASSES
                p = jnp.broadcast_to(pb[slot][pl.ds(h, 1), _tile(tt)], (8, 128))
                if CHAIN and tt == 0 and ps > 0:
                    p = jnp.where(flag, accs[0], p)
                new = []
                for g in range(gp):
                    f = _bf(vbuf[i * G + ps * gp + g, :, _tile(tt)]).astype(F32)
                    new += [f[:8] * p, f[8:] * p]
                accs = new if tt == 0 else [a + b for a, b in zip(accs, new)]
                hist.append(accs)
                if tt == nv - 1:
                    ab[slot][ps * gp * 16:(ps + 1) * gp * 16, :] = jnp.concatenate(accs, axis=0)

        def finish(x, dma):
            slot = (NP - 1) % 2
            cols = [key_sum(ab[slot][_tile(c), :]) for c in range(PW // 128)]
            o = normalize(cols, lp[...], slot, bd)
            y = jnp.concatenate([out_tile(o, NP - 1, c) for c in range(D // 128)], axis=1)
            x = x + jnp.sum(yb[...] + y, axis=0, keepdims=True)
            xc, rs = _center(x)
            if dma:
                wait(c_w1)
            hid = jnp.dot(xc.astype(BF16), w1b[...], preferred_element_type=F32) * rs
            hid = hid + b1b[...].astype(F32).reshape(1, FF)
            hid = jax.nn.gelu(hid, approximate=True).astype(BF16)
            x = x + b2b[...].astype(F32).reshape(1, D)
            for c in range(W2_CHUNKS):
                if dma:
                    wait(c_w2[c])
                x = x + jnp.dot(hid[:, c * f2:(c + 1) * f2], w2b[c * f2:(c + 1) * f2, :],
                                preferred_element_type=F32)
            return x

        def layer(li, x):
            xc, rs = _center(x)
            xc, rs = _pack(xc), rs * exp_scale
            for c in range(PW // 128):
                q_tile(xc, rs, 0, c, 0)
            q = _pack(q0[...])
            mx = None
            for t in range(nt):
                s = qk_tile(q, 0, t)
                mx = s if t == 0 else jnp.maximum(mx, s)
            for c in range(PW // 128):
                q_tile(xc, rs, 1, c, 1)
            m = jnp.max(mx, axis=-1, keepdims=True)
            lc[...] = sum(exp_tile(m, t, 0) for t in range(nt))
            yb[...] = jnp.zeros(yb.shape, F32)

            def body(it, carry):
                for u in range(2):
                    @pl.when(one[u] > 0)
                    def _():
                        pair_step(xc, rs, 2 * it + u, u, MAIN, vt_main.at[2 * it + u], True, True, u == 0)
                return carry

            lax.fori_loop(0, NP // 2 - 1, body, 0)

            @pl.when(li == 0)
            def _():
                wait(c_v1)
                transpose_v(NP - 2, vt_pen, PENULT[0])
                transpose_v(NP - 1, vt_last, LAST[0])
                wait(c_tail)

            @pl.when(one[2] > 0)
            def _():
                pair_step(xc, rs, NP - 2, 0, PENULT, vt_pen, True, False, False)

            @pl.when(one[3] > 0)
            def _():
                pair_step(xc, rs, NP - 1, 1, LAST, vt_last, False, False, False)

            return lax.cond(li == 0, lambda: finish(x, True), lambda: finish(x, False))

        wait(c_v0)

        @pl.loop(0, NP - 2)
        def _(j):
            transpose_v(j, vt_main.at[j], MAIN[0])

        wait(c_head)
        x0 = jnp.broadcast_to(xb[...].astype(F32), (8, D))
        o_ref[...] = lax.fori_loop(0, NL, layer, x0)[0:1].astype(o_ref.dtype)

    return kernel, 18 + W2_CHUNKS


@jax.jit
def pallas_interleave_layers__sliding_block_cached__dense_activation_gelu__decode_kernel(
    A_x: jax.Array,
    A_k_cache: jax.Array,
    A_v_cache: jax.Array,
    A_wq: jax.Array,
    A_wo: jax.Array,
    B_x: jax.Array,
    B_w1: jax.Array,
    B_b1: jax.Array,
    B_w2: jax.Array,
    B_b2: jax.Array,
):
    del B_x
    sk = A_k_cache.shape[2]
    win = min(4096, max(256, sk // 4))
    rows = H * DH
    kt = jnp.swapaxes(A_k_cache, 2, 3).reshape(rows // 16, 2, 8, sk)
    vt = jnp.swapaxes(A_v_cache, 2, 3).reshape(rows // 16, 2, 8, sk)
    wq = A_wq.reshape(D // 16, 2, 8, rows)
    wo = A_wo.reshape(rows // 16, 2, 8, D)
    kernel, n_sems = _make_kernel(sk, win)
    out = pl.pallas_call(
        kernel,
        out_shape=jax.ShapeDtypeStruct((1, D), A_x.dtype),
        in_specs=[pl.BlockSpec(memory_space=pl.ANY)] * 9,
        out_specs=pl.BlockSpec(memory_space=pltpu.VMEM),
        scratch_shapes=[
            pltpu.VMEM((rows // 16, 8, win), U32),
            pltpu.VMEM((rows // 16, 8, win), U32),
            pltpu.VMEM((D // 16, 8, rows), U32),
            pltpu.VMEM((rows // 16, 8, D), U32),
            pltpu.VMEM((D, FF), BF16),
            pltpu.VMEM((FF, D), BF16),
            pltpu.VMEM((1, D), BF16),
            pltpu.VMEM((FF,), BF16),
            pltpu.VMEM((D,), BF16),
            pltpu.VMEM((NP - 2, MAIN[0] * 64, PW), U32),
            pltpu.VMEM((PENULT[0] * 64, PW), U32),
            pltpu.VMEM((LAST[0] * 64, PW), U32),
            *[pltpu.VMEM((8, PW), F32)] * 2,
            pltpu.VMEM((8, win), F32),
            *[pltpu.VMEM((8, win), F32)] * 2,
            *[pltpu.VMEM((PW, 128), F32)] * 2,
            *[pltpu.VMEM((8, PW), F32)] * 2,
            *[pltpu.VMEM((8, 128), F32)] * 2,
            pltpu.VMEM((8, 128), F32),
            pltpu.VMEM((8, D), F32),
            pltpu.SMEM((4,), jnp.int32),
            pltpu.SemaphoreType.DMA((n_sems,)),
        ],
        compiler_params=pltpu.CompilerParams(vmem_limit_bytes=128 * 2**20),
        name="attn_ffn_decode",
    )(A_x.reshape(1, D), kt, vt, wq, wo, B_w1, B_b1, B_w2, B_b2)
    return out.reshape(A_x.shape)
```

```python
import numpy as np
import jax
import jax.numpy as jnp
from jax import lax
import jax.experimental.pallas as pl
import jax.experimental.pallas.tpu as pltpu

F32 = jnp.float32
BF16 = jnp.bfloat16
U32 = jnp.uint32

D = 640
H = 32
DH = 192
FF = 1536
NP = H // 2
PW = 2 * DH
G = PW // 16
NL = 2
W2_CHUNKS = 4

PASSES = 12
CHAIN = False
PVJ = 4
PVFIRST = False
MAIN = (0, 4, 30, 32)
PENULT = (4, 4, 30, 32)
LAST = (18, 0, 30, 16)


def _bf(w):
    return pltpu.bitcast(w, BF16)


def _pack(v):
    return pltpu.bitcast(jnp.concatenate([v, v], axis=0).astype(BF16), U32)


def _mm(lhs, w):
    return jnp.dot(_bf(lhs), _bf(w), preferred_element_type=F32)[:8]


def _center(x):
    c = x - jnp.mean(x, axis=-1, keepdims=True)
    v = jnp.mean(c * c, axis=-1, keepdims=True)
    return c, 1.0 / jnp.sqrt(v + 1e-5)


def _tile(t):
    return slice(t * 128, (t + 1) * 128)


def _make_kernel(sk, win):
    nt = win // 128
    f2 = FF // W2_CHUNKS
    gp = G // PASSES
    exp_scale = np.float32(DH ** -0.5 * np.log2(np.e))

    def kernel(x_hbm, k_hbm, v_hbm, wq_hbm, wo_hbm, w1_hbm, b1_hbm, w2_hbm, b2_hbm,
               o_ref,
               kbuf, vbuf, wqb, wob, w1b, w2b, xb, b1b, b2b,
               vt_pen, vt_last, q0, q1, sb, p0, p1, a0, a1, e0, e1, lp, lc, zb, yb, one, sems):
        qb, pb, ab, eb = (q0, q1), (p0, p1), (a0, a1), (e0, e1)

        copies = []

        def copy(src, dst):
            copies.append(pltpu.make_async_copy(src, dst, sems.at[len(copies)]))
            return [copies[-1]]

        def halves(src, dst, g0, g1, cols):
            s = src.bitcast(U32)
            rows = pl.ds(g0, g1 - g0)
            return (copy(s.at[rows, 0, :, cols], dst.at[rows, pl.ds(0, 4), :])
                    + copy(s.at[rows, 1, :, cols], dst.at[rows, pl.ds(4, 4), :]))

        window = pl.ds(sk - win, win)
        c_head = (halves(k_hbm, kbuf, 0, (NP - 1) * G, window)
                  + halves(v_hbm, vbuf, 0, (NP - 2) * G, window)
                  + halves(wq_hbm, wqb, 0, D // 16, pl.ds(0, H * DH))
                  + halves(wo_hbm, wob, 0, (NP - 3) * G, pl.ds(0, D))
                  + copy(x_hbm, xb) + copy(b1_hbm, b1b) + copy(b2_hbm, b2b))
        c_v1 = halves(v_hbm, vbuf, (NP - 2) * G, NP * G, window)
        c_tail = (halves(k_hbm, kbuf, (NP - 1) * G, NP * G, window)
                  + halves(wo_hbm, wob, (NP - 3) * G, NP * G, pl.ds(0, D)))
        c_w1 = copy(w1_hbm, w1b)
        c_w2 = [copy(w2_hbm.at[pl.ds(i * f2, f2)], w2b.at[pl.ds(i * f2, f2)])
                for i in range(W2_CHUNKS)]
        for c in copies:
            c.start()

        def wait(cs):
            for c in cs:
                c.wait()

        zb[...] = jnp.zeros(zb.shape, F32)
        a1[...] = jnp.zeros(a1.shape, F32)
        lp[...] = jnp.ones(lp.shape, F32)
        for u in range(4):
            one[u] = 1

        row = lax.broadcasted_iota(jnp.int32, (8, PW), 0)
        lane = lax.broadcasted_iota(jnp.int32, (8, PW), 1)
        bd = ((row == 0) & (lane < DH)) | ((row == 1) & (lane >= DH))

        def q_tile(xc, rs, j, c, slot):
            start = j * PW + c * 128
            if not isinstance(start, int):
                start = pl.multiple_of(start, 128)
            q = _mm(xc, wqb[:, :, pl.ds(start, 128)].reshape(D // 2, 128)) * rs
            qb[slot][:, _tile(c)] = jnp.where(bd[:, _tile(c)], q, 0.0)

        def qk_tile(q, j, t):
            s = _mm(q, kbuf[pl.ds(j * G, G), :, _tile(t)].reshape(PW // 2, 128))
            sb[:, _tile(t)] = s
            return s

        def exp_tile(m, t, slot):
            p = jnp.exp2(sb[:, _tile(t)] - m)
            pb[slot][:, _tile(t)] = p
            return p

        def key_sum(a):
            a = jnp.sum(a.T.reshape(16, 8, 128), axis=0)
            return jnp.broadcast_to(jnp.sum(a, axis=0, keepdims=True), (8, 128))

        def normalize(cols, l, slot, mask, extra):
            o = jnp.concatenate(cols, axis=1)
            if extra:
                o = o + eb[slot][...]
            return _pack(jnp.where(mask, o / jnp.sum(l, axis=-1, keepdims=True), 0.0))

        def out_tile(o, j, c):
            return _mm(o, wob[pl.ds(j * G, G), :, _tile(c)].reshape(PW // 2, 128))

        def transpose_v(j, vt, n):
            for t in range(n):
                w = _bf(vbuf[pl.ds(j * G, G), :, _tile(nt - n + t)].reshape(PW // 2, 128))
                vt[t * 64:(t + 1) * 64, :] = pltpu.bitcast(w.T, U32)

        def pair_step(xc, rs, i, slot, cfg, vt, do_qk, do_q, maybe_first):
            mxu_tiles, gate, tail, tstep = cfg
            nv = nt - mxu_tiles
            ns = PASSES * nv
            flag = zb[...] > 0.0
            l_prev = lp[...]
            lp[...] = lc[...]
            hist = []
            st = dict(n=0, l=None, mx=None, cols=[])
            if do_qk:
                st["q"] = _pack(qb[1 - slot][...])

            def gated(v, pos):
                if pos <= gate:
                    return v
                st["n"] += 1
                a = hist[pos - 1 - gate][st["n"] % (2 * gp)]
                g = jnp.where(flag, pltpu.bitcast(a, v.dtype), v[:8, :128])
                if v.shape[1] > 128:
                    return jnp.concatenate([g, v[:, 128:]], axis=1)
                return g if v.shape[0] == 8 else jnp.concatenate([g, v[8:]], axis=0)

            def job_qk(t, pos):
                s = qk_tile(gated(st["q"], pos), i + 1, t)
                st["mx"] = s if t == 0 else jnp.maximum(st["mx"], s)

            def job_exp(t, pos):
                if t == 0:
                    st["m"] = jnp.max(st["mx"], axis=-1, keepdims=True)
                p = exp_tile(st["m"], t, 1 - slot)
                st["l"] = p if t == 0 else st["l"] + p
                if t == nt - 1:
                    lc[...] = st["l"]

            def job_q(c, pos):
                q_tile(gated(xc, pos), rs, i + 2, c, slot)

            def job_t(c, pos):
                st["cols"].append(key_sum(gated(ab[1 - slot][_tile(c), :], pos)))
                if c == PW // 128 - 1:
                    mask = bd & (i > 0) if maybe_first else bd
                    st["o"] = normalize(st["cols"], l_prev, 1 - slot, mask, not do_qk)

            def job_o(c, pos):
                j = jnp.maximum(i - 1, 0) if maybe_first else i - 1
                yb[:, _tile(c)] += out_tile(gated(st["o"], pos), j, c)

            def job_pv(arg, pos):
                c, t0, t1 = arg
                lhs = _pack(pb[slot][:, (nv + t0) * 128:(nv + t1) * 128])
                e = _mm(gated(lhs, pos), vt[t0 * 64:t1 * 64, _tile(c)])
                st["e"] = e if t0 == 0 else st["e"] + e
                if t1 == mxu_tiles:
                    eb[slot][:, _tile(c)] = st["e"]

            qk = [(job_qk, t, 3) for t in range(nt)] if do_qk else []
            out = [(job_o, c, 3) for c in range(D // 128)]
            pv = [(job_pv, (c, t, min(t + PVJ, mxu_tiles)), min(PVJ, mxu_tiles - t))
                  for c in range(PW // 128) for t in range(0, mxu_tiles, PVJ)]
            qp = [(job_q, c, 5) for c in range(PW // 128)] if do_q else []
            jobs = (pv + qk + out + qp if PVFIRST else qk + pv + out + qp)
            total = sum(j[2] for j in jobs)
            at, done = {}, 0
            for c in range(PW // 128):
                at.setdefault(c * tstep, []).append((job_t, c))
            for fn, arg, cost in jobs:
                at.setdefault(done * (ns - tail) // total, []).append((fn, arg))
                done += cost
            if do_qk:
                for t in range(nt):
                    at.setdefault(ns - nt + t, []).append((job_exp, t))

            accs = None
            for pos in range(ns):
                ps, tt = divmod(pos, nv)
                for fn, arg in at.get(pos, []):
                    fn(arg, pos)
                h = ps * 2 // PASSES
                p = jnp.broadcast_to(pb[slot][pl.ds(h, 1), _tile(tt)], (8, 128))
                if CHAIN and tt == 0 and ps > 0:
                    p = jnp.where(flag, accs[0], p)
                new = []
                for g in range(gp):
                    f = _bf(vbuf[i * G + ps * gp + g, :, _tile(tt)]).astype(F32)
                    new += [f[:8] * p, f[8:] * p]
                accs = new if tt == 0 else [a + b for a, b in zip(accs, new)]
                hist.append(accs)
                if tt == nv - 1:
                    ab[slot][ps * gp * 16:(ps + 1) * gp * 16, :] = jnp.concatenate(accs, axis=0)

        def finish(x, dma):
            slot = (NP - 1) % 2
            cols = [key_sum(ab[slot][_tile(c), :]) for c in range(PW // 128)]
            o = normalize(cols, lp[...], slot, bd, True)
            y = jnp.concatenate([out_tile(o, NP - 1, c) for c in range(D // 128)], axis=1)
            x = x + jnp.sum(yb[...] + y, axis=0, keepdims=True)
            xc, rs = _center(x)
            if dma:
                wait(c_w1)
            hid = jnp.dot(xc.astype(BF16), w1b[...], preferred_element_type=F32) * rs
            hid = hid + b1b[...].astype(F32).reshape(1, FF)
            hid = jax.nn.gelu(hid, approximate=True).astype(BF16)
            x = x + b2b[...].astype(F32).reshape(1, D)
            for c in range(W2_CHUNKS):
                if dma:
                    wait(c_w2[c])
                x = x + jnp.dot(hid[:, c * f2:(c + 1) * f2], w2b[c * f2:(c + 1) * f2, :],
                                preferred_element_type=F32)
            return x

        def layer(li, x):
            xc, rs = _center(x)
            xc, rs = _pack(xc), rs * exp_scale
            for c in range(PW // 128):
                q_tile(xc, rs, 0, c, 0)
            q = _pack(q0[...])
            mx = None
            for t in range(nt):
                s = qk_tile(q, 0, t)
                mx = s if t == 0 else jnp.maximum(mx, s)
            for c in range(PW // 128):
                q_tile(xc, rs, 1, c, 1)
            m = jnp.max(mx, axis=-1, keepdims=True)
            lc[...] = sum(exp_tile(m, t, 0) for t in range(nt))
            yb[...] = jnp.zeros(yb.shape, F32)

            def body(it, carry):
                for u in range(2):
                    @pl.when(one[u] > 0)
                    def _():
                        pair_step(xc, rs, 2 * it + u, u, MAIN, None, True, True, u == 0)
                return carry

            lax.fori_loop(0, NP // 2 - 1, body, 0)

            @pl.when(li == 0)
            def _():
                wait(c_v1)
                transpose_v(NP - 2, vt_pen, PENULT[0])
                transpose_v(NP - 1, vt_last, LAST[0])
                wait(c_tail)

            @pl.when(one[2] > 0)
            def _():
                pair_step(xc, rs, NP - 2, 0, PENULT, vt_pen, True, False, False)

            @pl.when(one[3] > 0)
            def _():
                pair_step(xc, rs, NP - 1, 1, LAST, vt_last, False, False, False)

            return lax.cond(li == 0, lambda: finish(x, True), lambda: finish(x, False))

        wait(c_head)
        x0 = jnp.broadcast_to(xb[...].astype(F32), (8, D))
        o_ref[...] = lax.fori_loop(0, NL, layer, x0)[0:1].astype(o_ref.dtype)

    return kernel, 18 + W2_CHUNKS


@jax.jit
def pallas_interleave_layers__sliding_block_cached__dense_activation_gelu__decode_kernel(
    A_x: jax.Array,
    A_k_cache: jax.Array,
    A_v_cache: jax.Array,
    A_wq: jax.Array,
    A_wo: jax.Array,
    B_x: jax.Array,
    B_w1: jax.Array,
    B_b1: jax.Array,
    B_w2: jax.Array,
    B_b2: jax.Array,
):
    del B_x
    sk = A_k_cache.shape[2]
    win = min(4096, max(256, sk // 4))
    rows = H * DH
    kt = jnp.swapaxes(A_k_cache, 2, 3).reshape(rows // 16, 2, 8, sk)
    vt = jnp.swapaxes(A_v_cache, 2, 3).reshape(rows // 16, 2, 8, sk)
    wq = A_wq.reshape(D // 16, 2, 8, rows)
    wo = A_wo.reshape(rows // 16, 2, 8, D)
    kernel, n_sems = _make_kernel(sk, win)
    out = pl.pallas_call(
        kernel,
        out_shape=jax.ShapeDtypeStruct((1, D), A_x.dtype),
        in_specs=[pl.BlockSpec(memory_space=pl.ANY)] * 9,
        out_specs=pl.BlockSpec(memory_space=pltpu.VMEM),
        scratch_shapes=[
            pltpu.VMEM((rows // 16, 8, win), U32),
            pltpu.VMEM((rows // 16, 8, win), U32),
            pltpu.VMEM((D // 16, 8, rows), U32),
            pltpu.VMEM((rows // 16, 8, D), U32),
            pltpu.VMEM((D, FF), BF16),
            pltpu.VMEM((FF, D), BF16),
            pltpu.VMEM((1, D), BF16),
            pltpu.VMEM((FF,), BF16),
            pltpu.VMEM((D,), BF16),
            pltpu.VMEM((PENULT[0] * 64, PW), U32),
            pltpu.VMEM((LAST[0] * 64, PW), U32),
            *[pltpu.VMEM((8, PW), F32)] * 2,
            pltpu.VMEM((8, win), F32),
            *[pltpu.VMEM((8, win), F32)] * 2,
            *[pltpu.VMEM((PW, 128), F32)] * 2,
            *[pltpu.VMEM((8, PW), F32)] * 2,
            *[pltpu.VMEM((8, 128), F32)] * 2,
            pltpu.VMEM((8, 128), F32),
            pltpu.VMEM((8, D), F32),
            pltpu.SMEM((4,), jnp.int32),
            pltpu.SemaphoreType.DMA((n_sems,)),
        ],
        compiler_params=pltpu.CompilerParams(vmem_limit_bytes=126 * 2**20),
        name="attn_ffn_decode",
    )(A_x.reshape(1, D), kt, vt, wq, wo, B_w1, B_b1, B_w2, B_b2)
    return out.reshape(A_x.shape)
```

```python
import numpy as np
import jax
import jax.numpy as jnp
from jax import lax
import jax.experimental.pallas as pl
import jax.experimental.pallas.tpu as pltpu

F32 = jnp.float32
BF16 = jnp.bfloat16
U32 = jnp.uint32

D = 640
H = 32
DH = 192
FF = 1536
NP = H // 2
PW = 2 * DH
G = PW // 16
R = PW // 8
SPLIT = 10
NL = 2
W2_CHUNKS = 4

PASSES = 24
TREE = False
PVJ = 4
PVFIRST = False
MAIN = (0, 4, 30, 32)
PENULT = (4, 4, 30, 32)
LAST = (18, 0, 30, 16)


def _bf(w):
    return pltpu.bitcast(w, BF16)


def _pack(v):
    return pltpu.bitcast(jnp.concatenate([v, v], axis=0).astype(BF16), U32)


def _mm(lhs, w):
    return jnp.dot(_bf(lhs), _bf(w), preferred_element_type=F32)[:8]


def _center(x):
    c = x - jnp.mean(x, axis=-1, keepdims=True)
    v = jnp.mean(c * c, axis=-1, keepdims=True)
    return c, 1.0 / jnp.sqrt(v + 1e-5)


def _tile(t):
    return slice(t * 128, (t + 1) * 128)


def _make_kernel(sk, win):
    nt = win // 128
    f2 = FF // W2_CHUNKS
    gp = R // PASSES
    exp_scale = np.float32(DH ** -0.5 * np.log2(np.e))

    def kernel(x_hbm, k_hbm, v_hbm, wq_hbm, wo_hbm, w1_hbm, b1_hbm, w2_hbm, b2_hbm,
               o_ref,
               kbuf, vbuf, wqb, wob, w1b, w2b, xb, b1b, b2b,
               vt_pen, vt_last, q0, q1, sb, p0, p1, a0, a1, e0, e1, lp, lc, zb, yb, one, sems):
        qb, pb, ab, eb = (q0, q1), (p0, p1), (a0, a1), (e0, e1)

        copies = []

        def copy(src, dst):
            copies.append(pltpu.make_async_copy(src, dst, sems.at[len(copies)]))
            return [copies[-1]]

        def cache(src, j0, j1):
            rows = pl.ds(j0 * R, (j1 - j0) * R)
            return copy(src.at[rows, :, pl.ds(sk - win, win)], vbuf.at[rows])

        def start(cs):
            for c in cs:
                c.start()

        def wait(cs):
            for c in cs:
                c.wait()

        def repack(dst, d0, n, dst_cols, s0, src_cols):
            @pl.loop(0, n)
            def _(g):
                v = vbuf[pl.ds(s0 + 2 * g, 2), :, src_cols]
                dst[d0 + g, :, dst_cols] = pltpu.bitcast(v.reshape(16, v.shape[-1]), U32)

        wq_parts = [(c, min(win, H * DH - c), SPLIT * R + k * (D // 8))
                    for k, c in enumerate(range(0, H * DH, win))]
        wo_row = wq_parts[-1][2] + D // 8
        wo_parts = win // D
        wo_n = NP * R // wo_parts
        assert wo_n * wo_parts == NP * R and wo_row + wo_n <= NP * R
        c_w = copy(x_hbm, xb) + copy(b1_hbm, b1b) + copy(b2_hbm, b2b)
        for c, n, r in wq_parts:
            c_w += copy(wq_hbm.at[:, :, pl.ds(c, n)], vbuf.at[pl.ds(r, D // 8), :, pl.ds(0, n)])
        for k in range(wo_parts):
            c_w += copy(wo_hbm.at[pl.ds(k * wo_n, wo_n)],
                        vbuf.at[pl.ds(wo_row, wo_n), :, pl.ds(k * D, D)])
        c_k0, c_k1 = cache(k_hbm, 0, SPLIT), cache(k_hbm, SPLIT, NP)
        c_v0, c_v1 = cache(v_hbm, 0, SPLIT), cache(v_hbm, SPLIT, NP - 2)
        c_v2 = cache(v_hbm, NP - 2, NP)
        c_w1 = copy(w1_hbm, w1b)
        c_w2 = [copy(w2_hbm.at[pl.ds(i * f2, f2)], w2b.at[pl.ds(i * f2, f2)])
                for i in range(W2_CHUNKS)]

        start(c_w[3:] + c_w[:3] + c_k0)
        wait(c_w)
        for c, n, r in wq_parts:
            repack(wqb, 0, D // 16, slice(c, c + n), r, slice(0, n))
        for k in range(wo_parts):
            repack(wob, k * wo_n // 2, wo_n // 2, slice(0, D), wo_row, slice(k * D, (k + 1) * D))
        start(c_k1)
        wait(c_k0)
        repack(kbuf, 0, SPLIT * G, slice(0, win), 0, slice(0, win))
        start(c_v0)
        wait(c_k1)
        repack(kbuf, SPLIT * G, (NP - SPLIT) * G, slice(0, win), SPLIT * R, slice(0, win))
        start(c_v1 + c_v2 + c_w1 + sum(c_w2, []))

        zb[...] = jnp.zeros(zb.shape, F32)
        a1[...] = jnp.zeros(a1.shape, F32)
        lp[...] = jnp.ones(lp.shape, F32)
        for u in range(4):
            one[u] = 1

        row = lax.broadcasted_iota(jnp.int32, (8, PW), 0)
        lane = lax.broadcasted_iota(jnp.int32, (8, PW), 1)
        bd = ((row == 0) & (lane < DH)) | ((row == 1) & (lane >= DH))

        def q_tile(xc, rs, j, c, slot):
            start = j * PW + c * 128
            if not isinstance(start, int):
                start = pl.multiple_of(start, 128)
            q = _mm(xc, wqb[:, :, pl.ds(start, 128)].reshape(D // 2, 128)) * rs
            qb[slot][:, _tile(c)] = jnp.where(bd[:, _tile(c)], q, 0.0)

        def qk_tile(q, j, t):
            s = _mm(q, kbuf[pl.ds(j * G, G), :, _tile(t)].reshape(PW // 2, 128))
            sb[:, _tile(t)] = s
            return s

        def exp_tile(m, t, slot):
            p = jnp.exp2(sb[:, _tile(t)] - m)
            pb[slot][:, _tile(t)] = p
            return p

        def key_sum(a):
            a = jnp.sum(a.T.reshape(16, 8, 128), axis=0)
            return jnp.broadcast_to(jnp.sum(a, axis=0, keepdims=True), (8, 128))

        def normalize(cols, l, slot, mask, extra):
            o = jnp.concatenate(cols, axis=1)
            if extra:
                o = o + eb[slot][...]
            return _pack(jnp.where(mask, o / jnp.sum(l, axis=-1, keepdims=True), 0.0))

        def out_tile(o, j, c):
            return _mm(o, wob[pl.ds(j * G, G), :, _tile(c)].reshape(PW // 2, 128))

        def transpose_v(j, vt, n):
            for t in range(n):
                w = vbuf[pl.ds(j * R, R), :, _tile(nt - n + t)].reshape(PW, 128)
                vt[t * 64:(t + 1) * 64, :] = pltpu.bitcast(w.T, U32)

        def pair_step(xc, rs, i, slot, cfg, vt, do_qk, do_q, maybe_first):
            mxu_tiles, gate, tail, tstep = cfg
            nv = nt - mxu_tiles
            ns = PASSES * nv // 2
            flag = zb[...] > 0.0
            l_prev = lp[...]
            lp[...] = lc[...]
            hist = []
            st = dict(n=0, l=None, mx=None, cols=[])
            if do_qk:
                st["q"] = _pack(qb[1 - slot][...])

            def gated(v, pos):
                if pos <= gate:
                    return v
                st["n"] += 1
                a = hist[pos - 1 - gate]
                a = a[st["n"] % len(a)]
                g = jnp.where(flag, pltpu.bitcast(a, v.dtype), v[:8, :128])
                if v.shape[1] > 128:
                    return jnp.concatenate([g, v[:, 128:]], axis=1)
                return g if v.shape[0] == 8 else jnp.concatenate([g, v[8:]], axis=0)

            def job_qk(t, pos):
                s = qk_tile(gated(st["q"], pos), i + 1, t)
                st["mx"] = s if t == 0 else jnp.maximum(st["mx"], s)

            def job_exp(t, pos):
                if t == 0:
                    st["m"] = jnp.max(st["mx"], axis=-1, keepdims=True)
                p = exp_tile(st["m"], t, 1 - slot)
                st["l"] = p if t == 0 else st["l"] + p
                if t == nt - 1:
                    lc[...] = st["l"]

            def job_q(c, pos):
                q_tile(gated(xc, pos), rs, i + 2, c, slot)

            def job_t(c, pos):
                st["cols"].append(key_sum(gated(ab[1 - slot][_tile(c), :], pos)))
                if c == PW // 128 - 1:
                    mask = bd & (i > 0) if maybe_first else bd
                    st["o"] = normalize(st["cols"], l_prev, 1 - slot, mask, not do_qk)

            def job_o(c, pos):
                j = jnp.maximum(i - 1, 0) if maybe_first else i - 1
                yb[:, _tile(c)] += out_tile(gated(st["o"], pos), j, c)

            def job_pv(arg, pos):
                c, t0, t1 = arg
                lhs = _pack(pb[slot][:, (nv + t0) * 128:(nv + t1) * 128])
                e = _mm(gated(lhs, pos), vt[t0 * 64:t1 * 64, _tile(c)])
                st["e"] = e if t0 == 0 else st["e"] + e
                if t1 == mxu_tiles:
                    eb[slot][:, _tile(c)] = st["e"]

            qk = [(job_qk, t, 3) for t in range(nt)] if do_qk else []
            out = [(job_o, c, 3) for c in range(D // 128)]
            pv = [(job_pv, (c, t, min(t + PVJ, mxu_tiles)), min(PVJ, mxu_tiles - t))
                  for c in range(PW // 128) for t in range(0, mxu_tiles, PVJ)]
            qp = [(job_q, c, 5) for c in range(PW // 128)] if do_q else []
            jobs = (pv + qk + out + qp if PVFIRST else qk + pv + out + qp)
            total = sum(j[2] for j in jobs)
            at, done = {}, 0
            for c in range(PW // 128):
                at.setdefault(c * tstep, []).append((job_t, c))
            for fn, arg, cost in jobs:
                at.setdefault(done * (ns - tail) // total, []).append((fn, arg))
                done += cost
            if do_qk:
                for t in range(nt):
                    at.setdefault(ns - nt + t, []).append((job_exp, t))

            accs = None
            for pos in range(ns):
                ps, tt = divmod(pos, nv // 2)
                for fn, arg in at.get(pos, []):
                    fn(arg, pos)
                keys = slice(tt * 256, (tt + 1) * 256)
                pa, pc = [jnp.broadcast_to(pb[slot][pl.ds(ps * 2 // PASSES, 1), _tile(t)], (8, 128))
                          for t in (2 * tt, 2 * tt + 1)]
                new = []
                for g in range(gp):
                    f = vbuf[i * R + ps * gp + g, :, keys].astype(F32)
                    fa, fc = f[:, :128] * pa, f[:, 128:] * pc
                    new += [fa + fc] if TREE else [fa, fc]
                accs = new if tt == 0 else [a + b for a, b in zip(accs, new)]
                hist.append(accs)
                if tt == nv // 2 - 1:
                    done = accs if TREE else [a + b for a, b in zip(accs[::2], accs[1::2])]
                    ab[slot][ps * gp * 8:(ps + 1) * gp * 8, :] = jnp.concatenate(done, axis=0)

        def finish(x, dma):
            slot = (NP - 1) % 2
            cols = [key_sum(ab[slot][_tile(c), :]) for c in range(PW // 128)]
            o = normalize(cols, lp[...], slot, bd, True)
            y = jnp.concatenate([out_tile(o, NP - 1, c) for c in range(D // 128)], axis=1)
            x = x + jnp.sum(yb[...] + y, axis=0, keepdims=True)
            xc, rs = _center(x)
            if dma:
                wait(c_w1)
            hid = jnp.dot(xc.astype(BF16), w1b[...], preferred_element_type=F32) * rs
            hid = hid + b1b[...].astype(F32).reshape(1, FF)
            hid = jax.nn.gelu(hid, approximate=True).astype(BF16)
            x = x + b2b[...].astype(F32).reshape(1, D)
            for c in range(W2_CHUNKS):
                if dma:
                    wait(c_w2[c])
                x = x + jnp.dot(hid[:, c * f2:(c + 1) * f2], w2b[c * f2:(c + 1) * f2, :],
                                preferred_element_type=F32)
            return x

        def layer(li, x):
            xc, rs = _center(x)
            xc, rs = _pack(xc), rs * exp_scale
            for c in range(PW // 128):
                q_tile(xc, rs, 0, c, 0)
            q = _pack(q0[...])
            mx = None
            for t in range(nt):
                s = qk_tile(q, 0, t)
                mx = s if t == 0 else jnp.maximum(mx, s)
            for c in range(PW // 128):
                q_tile(xc, rs, 1, c, 1)
            m = jnp.max(mx, axis=-1, keepdims=True)
            lc[...] = sum(exp_tile(m, t, 0) for t in range(nt))
            yb[...] = jnp.zeros(yb.shape, F32)

            def body(it, carry):
                @pl.when((li == 0) & (it == SPLIT // 2))
                def _():
                    wait(c_v1)

                for u in range(2):
                    @pl.when(one[u] > 0)
                    def _():
                        pair_step(xc, rs, 2 * it + u, u, MAIN, None, True, True, u == 0)
                return carry

            lax.fori_loop(0, NP // 2 - 1, body, 0)

            @pl.when(li == 0)
            def _():
                wait(c_v2)
                transpose_v(NP - 2, vt_pen, PENULT[0])
                transpose_v(NP - 1, vt_last, LAST[0])

            @pl.when(one[2] > 0)
            def _():
                pair_step(xc, rs, NP - 2, 0, PENULT, vt_pen, True, False, False)

            @pl.when(one[3] > 0)
            def _():
                pair_step(xc, rs, NP - 1, 1, LAST, vt_last, False, False, False)

            return lax.cond(li == 0, lambda: finish(x, True), lambda: finish(x, False))

        wait(c_v0)
        x0 = jnp.broadcast_to(xb[...].astype(F32), (8, D))
        o_ref[...] = lax.fori_loop(0, NL, layer, x0)[0:1].astype(o_ref.dtype)

    return kernel, 9 + -(-H * DH // win) + win // D + W2_CHUNKS


@jax.jit
def pallas_interleave_layers__sliding_block_cached__dense_activation_gelu__decode_kernel(
    A_x: jax.Array,
    A_k_cache: jax.Array,
    A_v_cache: jax.Array,
    A_wq: jax.Array,
    A_wo: jax.Array,
    B_x: jax.Array,
    B_w1: jax.Array,
    B_b1: jax.Array,
    B_w2: jax.Array,
    B_b2: jax.Array,
):
    del B_x
    sk = A_k_cache.shape[2]
    win = min(4096, max(256, sk // 4))
    rows = H * DH
    kt = jnp.swapaxes(A_k_cache, 2, 3).reshape(rows // 8, 8, sk)
    vt = jnp.swapaxes(A_v_cache, 2, 3).reshape(rows // 8, 8, sk)
    wq = A_wq.reshape(D // 8, 8, rows)
    wo = A_wo.reshape(rows // 8, 8, D)
    kernel, n_sems = _make_kernel(sk, win)
    out = pl.pallas_call(
        kernel,
        out_shape=jax.ShapeDtypeStruct((1, D), A_x.dtype),
        in_specs=[pl.BlockSpec(memory_space=pl.ANY)] * 9,
        out_specs=pl.BlockSpec(memory_space=pltpu.VMEM),
        scratch_shapes=[
            pltpu.VMEM((rows // 16, 8, win), U32),
            pltpu.VMEM((rows // 8, 8, win), BF16),
            pltpu.VMEM((D // 16, 8, rows), U32),
            pltpu.VMEM((rows // 16, 8, D), U32),
            pltpu.VMEM((D, FF), BF16),
            pltpu.VMEM((FF, D), BF16),
            pltpu.VMEM((1, D), BF16),
            pltpu.VMEM((FF,), BF16),
            pltpu.VMEM((D,), BF16),
            pltpu.VMEM((PENULT[0] * 64, PW), U32),
            pltpu.VMEM((LAST[0] * 64, PW), U32),
            *[pltpu.VMEM((8, PW), F32)] * 2,
            pltpu.VMEM((8, win), F32),
            *[pltpu.VMEM((8, win), F32)] * 2,
            *[pltpu.VMEM((PW, 128), F32)] * 2,
            *[pltpu.VMEM((8, PW), F32)] * 2,
            *[pltpu.VMEM((8, 128), F32)] * 2,
            pltpu.VMEM((8, 128), F32),
            pltpu.VMEM((8, D), F32),
            pltpu.SMEM((4,), jnp.int32),
            pltpu.SemaphoreType.DMA((n_sems,)),
        ],
        compiler_params=pltpu.CompilerParams(vmem_limit_bytes=126 * 2**20),
        name="attn_ffn_decode",
    )(A_x.reshape(1, D), kt, vt, wq, wo, B_w1, B_b1, B_w2, B_b2)
    return out.reshape(A_x.shape)
```

```python
import numpy as np
import jax
import jax.numpy as jnp
from jax import lax
import jax.experimental.pallas as pl
import jax.experimental.pallas.tpu as pltpu

F32 = jnp.float32
BF16 = jnp.bfloat16
U32 = jnp.uint32

D = 640
H = 32
DH = 192
FF = 1536
NP = H // 2
PW = 2 * DH
G = PW // 16
R = PW // 8
SPLIT = 10
NL = 2
W2_CHUNKS = 4

PASSES = 16
PVJ = 4
MAIN = (0, 0, 14, 32)
PENULT = (4, 2, 10, 21)
LAST = (18, 0, 20, 10)


def _bf(w):
    return pltpu.bitcast(w, BF16)


def _pack(v):
    return pltpu.bitcast(jnp.concatenate([v, v], axis=0).astype(BF16), U32)


def _mm(lhs, w):
    return jnp.dot(_bf(lhs), _bf(w), preferred_element_type=F32)[:8]


def _center(x):
    c = x - jnp.mean(x, axis=-1, keepdims=True)
    v = jnp.mean(c * c, axis=-1, keepdims=True)
    return c, 1.0 / jnp.sqrt(v + 1e-5)


def _tile(t):
    return slice(t * 128, (t + 1) * 128)


def _make_kernel(sk, win):
    nt = win // 128
    f2 = FF // W2_CHUNKS
    gp = R // PASSES
    exp_scale = np.float32(DH ** -0.5 * np.log2(np.e))

    def kernel(x_hbm, k_hbm, v_hbm, wq_hbm, wo_hbm, w1_hbm, b1_hbm, w2_hbm, b2_hbm,
               o_ref,
               kbuf, vbuf, wqb, wob, w1b, w2b, xb, b1b, b2b,
               vt_pen, vt_last, q0, q1, sb, p0, p1, a0, a1, e0, e1, lp, lc, zb, yb, one, sems):
        qb, pb, ab, eb = (q0, q1), (p0, p1), (a0, a1), (e0, e1)

        copies = []

        def copy(src, dst):
            copies.append(pltpu.make_async_copy(src, dst, sems.at[len(copies)]))
            return [copies[-1]]

        def cache(src, j0, j1):
            rows = pl.ds(j0 * R, (j1 - j0) * R)
            return copy(src.at[rows, :, pl.ds(sk - win, win)], vbuf.at[rows])

        def start(cs):
            for c in cs:
                c.start()

        def wait(cs):
            for c in cs:
                c.wait()

        def repack(dst, d0, n, dst_cols, s0, src_cols):
            @pl.loop(0, n)
            def _(g):
                v = vbuf[pl.ds(s0 + 2 * g, 2), :, src_cols]
                dst[d0 + g, :, dst_cols] = pltpu.bitcast(v.reshape(16, v.shape[-1]), U32)

        wq_parts = [(c, min(win, H * DH - c), SPLIT * R + k * (D // 8))
                    for k, c in enumerate(range(0, H * DH, win))]
        wo_row = wq_parts[-1][2] + D // 8
        wo_parts = win // D
        wo_n = NP * R // wo_parts
        assert wo_n * wo_parts == NP * R and wo_row + wo_n <= NP * R
        c_w = copy(x_hbm, xb) + copy(b1_hbm, b1b) + copy(b2_hbm, b2b)
        for c, n, r in wq_parts:
            c_w += copy(wq_hbm.at[:, :, pl.ds(c, n)], vbuf.at[pl.ds(r, D // 8), :, pl.ds(0, n)])
        for k in range(wo_parts):
            c_w += copy(wo_hbm.at[pl.ds(k * wo_n, wo_n)],
                        vbuf.at[pl.ds(wo_row, wo_n), :, pl.ds(k * D, D)])
        c_k0, c_k1 = cache(k_hbm, 0, SPLIT), cache(k_hbm, SPLIT, NP)
        c_v0, c_v1 = cache(v_hbm, 0, SPLIT), cache(v_hbm, SPLIT, NP - 2)
        c_v2 = cache(v_hbm, NP - 2, NP)
        c_w1 = copy(w1_hbm, w1b)
        c_w2 = [copy(w2_hbm.at[pl.ds(i * f2, f2)], w2b.at[pl.ds(i * f2, f2)])
                for i in range(W2_CHUNKS)]

        start(c_w[3:] + c_w[:3] + c_k0)
        wait(c_w)
        for c, n, r in wq_parts:
            repack(wqb, 0, D // 16, slice(c, c + n), r, slice(0, n))
        for k in range(wo_parts):
            repack(wob, k * wo_n // 2, wo_n // 2, slice(0, D), wo_row, slice(k * D, (k + 1) * D))
        start(c_k1)
        wait(c_k0)
        repack(kbuf, 0, SPLIT * G, slice(0, win), 0, slice(0, win))
        start(c_v0)
        wait(c_k1)
        repack(kbuf, SPLIT * G, (NP - SPLIT) * G, slice(0, win), SPLIT * R, slice(0, win))
        start(c_v1 + c_v2 + c_w1 + sum(c_w2, []))

        zb[...] = jnp.zeros(zb.shape, F32)
        a1[...] = jnp.zeros(a1.shape, F32)
        lp[...] = jnp.ones(lp.shape, F32)
        for u in range(4):
            one[u] = 1

        row = lax.broadcasted_iota(jnp.int32, (8, PW), 0)
        lane = lax.broadcasted_iota(jnp.int32, (8, PW), 1)
        bd = ((row == 0) & (lane < DH)) | ((row == 1) & (lane >= DH))

        def q_tile(xc, rs, j, c, slot):
            start = j * PW + c * 128
            if not isinstance(start, int):
                start = pl.multiple_of(start, 128)
            q = _mm(xc, wqb[:, :, pl.ds(start, 128)].reshape(D // 2, 128)) * rs
            qb[slot][:, _tile(c)] = jnp.where(bd[:, _tile(c)], q, 0.0)

        def qk_tile(q, j, t):
            s = _mm(q, kbuf[pl.ds(j * G, G), :, _tile(t)].reshape(PW // 2, 128))
            sb[:, _tile(t)] = s
            return s

        def exp_tile(m, t, slot):
            p = jnp.exp2(sb[:, _tile(t)] - m)
            pb[slot][:, _tile(t)] = p
            return p

        def key_sum(a):
            a = jnp.sum(a.T.reshape(16, 8, 128), axis=0)
            return jnp.broadcast_to(jnp.sum(a, axis=0, keepdims=True), (8, 128))

        def normalize(cols, l, slot, mask, extra):
            o = jnp.concatenate(cols, axis=1)
            if extra:
                o = o + eb[slot][...]
            return _pack(jnp.where(mask, o / jnp.sum(l, axis=-1, keepdims=True), 0.0))

        def out_tile(o, j, c):
            return _mm(o, wob[pl.ds(j * G, G), :, _tile(c)].reshape(PW // 2, 128))

        def transpose_v(j, vt, n):
            for t in range(n):
                w = vbuf[pl.ds(j * R, R), :, _tile(nt - n + t)].reshape(PW, 128)
                vt[t * 64:(t + 1) * 64, :] = pltpu.bitcast(w.T, U32)

        def pair_step(xc, rs, i, slot, cfg, vt, do_qk, do_q, maybe_first):
            mxu_tiles, gate, tail, tstep = cfg
            nv = nt - mxu_tiles
            ns = PASSES * nv // 2
            flag = zb[...] > 0.0
            l_prev = lp[...]
            lp[...] = lc[...]
            hist = []
            st = dict(n=0, l=None, mx=None, cols=[])
            if do_qk:
                st["q"] = _pack(qb[1 - slot][...])

            def gated(v, pos):
                if pos <= gate:
                    return v
                st["n"] += 1
                a = hist[pos - 1 - gate][st["n"] % gp]
                g = jnp.where(flag, pltpu.bitcast(a, v.dtype), v[:8, :128])
                if v.shape[1] > 128:
                    return jnp.concatenate([g, v[:, 128:]], axis=1)
                return g if v.shape[0] == 8 else jnp.concatenate([g, v[8:]], axis=0)

            def job_qk(t, pos):
                s = qk_tile(gated(st["q"], pos), i + 1, t)
                st["mx"] = s if t == 0 else jnp.maximum(st["mx"], s)

            def job_exp(t, pos):
                if t == 0:
                    st["m"] = jnp.max(st["mx"], axis=-1, keepdims=True)
                p = exp_tile(st["m"], t, 1 - slot)
                st["l"] = p if t == 0 else st["l"] + p
                if t == nt - 1:
                    lc[...] = st["l"]

            def job_q(c, pos):
                q_tile(gated(xc, pos), rs, i + 2, c, slot)

            def job_t(c, pos):
                st["cols"].append(key_sum(gated(ab[1 - slot][_tile(c), :], pos)))
                if c == PW // 128 - 1:
                    mask = bd & (i > 0) if maybe_first else bd
                    st["o"] = normalize(st["cols"], l_prev, 1 - slot, mask, not do_qk)

            def job_o(c, pos):
                j = jnp.maximum(i - 1, 0) if maybe_first else i - 1
                yb[:, _tile(c)] += out_tile(gated(st["o"], pos), j, c)

            def job_pv(arg, pos):
                c, t0, t1 = arg
                lhs = _pack(pb[slot][:, (nv + t0) * 128:(nv + t1) * 128])
                e = _mm(gated(lhs, pos), vt[t0 * 64:t1 * 64, _tile(c)])
                st["e"] = e if t0 == 0 else st["e"] + e
                if t1 == mxu_tiles:
                    eb[slot][:, _tile(c)] = st["e"]

            qk = [(job_qk, t, 3) for t in range(nt)] if do_qk else []
            out = [(job_o, c, 3) for c in range(D // 128)]
            pv = [(job_pv, (c, t, min(t + PVJ, mxu_tiles)), min(PVJ, mxu_tiles - t))
                  for c in range(PW // 128) for t in range(0, mxu_tiles, PVJ)]
            qp = [(job_q, c, 5) for c in range(PW // 128)] if do_q else []
            jobs = qk + pv + out + qp
            total = sum(j[2] for j in jobs)
            at, done = {}, 0
            for c in range(PW // 128):
                at.setdefault(c * tstep, []).append((job_t, c))
            for fn, arg, cost in jobs:
                at.setdefault(done * (ns - tail) // total, []).append((fn, arg))
                done += cost
            if do_qk:
                for t in range(nt):
                    at.setdefault(ns - nt + t, []).append((job_exp, t))

            accs = None
            for pos in range(ns):
                ps, tt = divmod(pos, nv // 2)
                for fn, arg in at.get(pos, []):
                    fn(arg, pos)
                keys = slice(tt * 256, (tt + 1) * 256)
                pa, pc = [jnp.broadcast_to(pb[slot][pl.ds(ps * 2 // PASSES, 1), _tile(t)], (8, 128))
                          for t in (2 * tt, 2 * tt + 1)]
                new = []
                for g in range(gp):
                    f = vbuf[i * R + ps * gp + g, :, keys].astype(F32)
                    new.append(f[:, :128] * pa + f[:, 128:] * pc)
                accs = new if tt == 0 else [a + b for a, b in zip(accs, new)]
                hist.append(accs)
                if tt == nv // 2 - 1:
                    ab[slot][ps * gp * 8:(ps + 1) * gp * 8, :] = jnp.concatenate(accs, axis=0)

        def finish(x, dma):
            slot = (NP - 1) % 2
            cols = [key_sum(ab[slot][_tile(c), :]) for c in range(PW // 128)]
            o = normalize(cols, lp[...], slot, bd, True)
            y = jnp.concatenate([out_tile(o, NP - 1, c) for c in range(D // 128)], axis=1)
            x = x + jnp.sum(yb[...] + y, axis=0, keepdims=True)
            xc, rs = _center(x)
            if dma:
                wait(c_w1)
            hid = jnp.dot(xc.astype(BF16), w1b[...], preferred_element_type=F32) * rs
            hid = hid + b1b[...].astype(F32).reshape(1, FF)
            hid = jax.nn.gelu(hid, approximate=True).astype(BF16)
            x = x + b2b[...].astype(F32).reshape(1, D)
            for c in range(W2_CHUNKS):
                if dma:
                    wait(c_w2[c])
                x = x + jnp.dot(hid[:, c * f2:(c + 1) * f2], w2b[c * f2:(c + 1) * f2, :],
                                preferred_element_type=F32)
            return x

        def layer(li, x):
            xc, rs = _center(x)
            xc, rs = _pack(xc), rs * exp_scale
            for c in range(PW // 128):
                q_tile(xc, rs, 0, c, 0)
            q = _pack(q0[...])
            mx = None
            for t in range(nt):
                s = qk_tile(q, 0, t)
                mx = s if t == 0 else jnp.maximum(mx, s)
            for c in range(PW // 128):
                q_tile(xc, rs, 1, c, 1)
            m = jnp.max(mx, axis=-1, keepdims=True)
            lc[...] = sum(exp_tile(m, t, 0) for t in range(nt))
            yb[...] = jnp.zeros(yb.shape, F32)

            def body(it, carry):
                @pl.when((li == 0) & (it == SPLIT // 2))
                def _():
                    wait(c_v1)

                for u in range(2):
                    @pl.when(one[u] > 0)
                    def _():
                        pair_step(xc, rs, 2 * it + u, u, MAIN, None, True, True, u == 0)
                return carry

            lax.fori_loop(0, NP // 2 - 1, body, 0)

            @pl.when(li == 0)
            def _():
                wait(c_v2)
                transpose_v(NP - 2, vt_pen, PENULT[0])
                transpose_v(NP - 1, vt_last, LAST[0])

            @pl.when(one[2] > 0)
            def _():
                pair_step(xc, rs, NP - 2, 0, PENULT, vt_pen, True, False, False)

            @pl.when(one[3] > 0)
            def _():
                pair_step(xc, rs, NP - 1, 1, LAST, vt_last, False, False, False)

            return lax.cond(li == 0, lambda: finish(x, True), lambda: finish(x, False))

        wait(c_v0)
        x0 = jnp.broadcast_to(xb[...].astype(F32), (8, D))
        o_ref[...] = lax.fori_loop(0, NL, layer, x0)[0:1].astype(o_ref.dtype)

    return kernel, 9 + -(-H * DH // win) + win // D + W2_CHUNKS


@jax.jit
def pallas_interleave_layers__sliding_block_cached__dense_activation_gelu__decode_kernel(
    A_x: jax.Array,
    A_k_cache: jax.Array,
    A_v_cache: jax.Array,
    A_wq: jax.Array,
    A_wo: jax.Array,
    B_x: jax.Array,
    B_w1: jax.Array,
    B_b1: jax.Array,
    B_w2: jax.Array,
    B_b2: jax.Array,
):
    del B_x
    sk = A_k_cache.shape[2]
    win = min(4096, max(256, sk // 4))
    rows = H * DH
    kt = jnp.swapaxes(A_k_cache, 2, 3).reshape(rows // 8, 8, sk)
    vt = jnp.swapaxes(A_v_cache, 2, 3).reshape(rows // 8, 8, sk)
    wq = A_wq.reshape(D // 8, 8, rows)
    wo = A_wo.reshape(rows // 8, 8, D)
    kernel, n_sems = _make_kernel(sk, win)
    out = pl.pallas_call(
        kernel,
        out_shape=jax.ShapeDtypeStruct((1, D), A_x.dtype),
        in_specs=[pl.BlockSpec(memory_space=pl.ANY)] * 9,
        out_specs=pl.BlockSpec(memory_space=pltpu.VMEM),
        scratch_shapes=[
            pltpu.VMEM((rows // 16, 8, win), U32),
            pltpu.VMEM((rows // 8, 8, win), BF16),
            pltpu.VMEM((D // 16, 8, rows), U32),
            pltpu.VMEM((rows // 16, 8, D), U32),
            pltpu.VMEM((D, FF), BF16),
            pltpu.VMEM((FF, D), BF16),
            pltpu.VMEM((1, D), BF16),
            pltpu.VMEM((FF,), BF16),
            pltpu.VMEM((D,), BF16),
            pltpu.VMEM((PENULT[0] * 64, PW), U32),
            pltpu.VMEM((LAST[0] * 64, PW), U32),
            *[pltpu.VMEM((8, PW), F32)] * 2,
            pltpu.VMEM((8, win), F32),
            *[pltpu.VMEM((8, win), F32)] * 2,
            *[pltpu.VMEM((PW, 128), F32)] * 2,
            *[pltpu.VMEM((8, PW), F32)] * 2,
            *[pltpu.VMEM((8, 128), F32)] * 2,
            pltpu.VMEM((8, 128), F32),
            pltpu.VMEM((8, D), F32),
            pltpu.SMEM((4,), jnp.int32),
            pltpu.SemaphoreType.DMA((n_sems,)),
        ],
        compiler_params=pltpu.CompilerParams(vmem_limit_bytes=126 * 2**20),
        name="attn_ffn_decode",
    )(A_x.reshape(1, D), kt, vt, wq, wo, B_w1, B_b1, B_w2, B_b2)
    return out.reshape(A_x.shape)
```
